```python
import jax
import jax.numpy as jnp

def _softmax(x, axis=-1):
    return jax.nn.softmax(x, axis=axis)

def _gelu(x):
    return jax.nn.gelu(x, approximate=True)

def _silu(x):
    return jax.nn.silu(x)

def _sigmoid(x):
    return jax.nn.sigmoid(x)

def _layernorm(x, axis=-1, eps=1e-05):
    m = jnp.mean(x, axis=axis, keepdims=True)
    v = jnp.var(x, axis=axis, keepdims=True)
    return (x - m) / jnp.sqrt(v + eps)

def _scatter_add(tgt, idx, src, axis=0):
    return tgt.at[idx].add(src)

def _segment_sum(src, seg, n):
    return jax.ops.segment_sum(src, seg, n)

class _Rng:

    def __init__(self, key):
        self._k = key

    def _next(self):
        self._k, sub = jax.random.split(self._k)
        return sub

    def normal(self, shape):
        return jax.random.normal(self._next(), shape, dtype=jnp.bfloat16)

    def randint(self, lo, hi, shape):
        return jax.random.randint(self._next(), shape, lo, hi, dtype=jnp.int32)

    def uniform(self, shape, lo=0.0, hi=1.0):
        return jax.random.uniform(self._next(), shape, jnp.bfloat16, lo, hi)

    def permutation(self, n):
        return jax.random.permutation(self._next(), n)
kernel_name = 'sequential_preLN__memory_aug_recurrent_mem_tr__mixer_s_mlp__prompt'

def setup_inputs():
    _rng = _Rng(jax.random.key(int.from_bytes(__import__("os").urandom(4), "little")))
    _w = lambda a: (lambda t: t.astype(jnp.bfloat16) if jnp.issubdtype(t.dtype, jnp.floating) else t)(jnp.asarray(a))

    def _A_setup():
        B, S, Dm = (1, 2048, 1024)
        H, Dh = (32, 128)
        M, seg = (8, 32)
        seg = min(seg, S)
        S = S // seg * seg
        return {'x': _w((lambda *s: _rng.normal(s) * 0.05)(B, S, Dm)), 'mem0': _w((lambda *s: _rng.normal(s) * 0.05)(B, M, Dm)), 'Wq': _w((lambda *s: _rng.normal(s) * 0.05)(Dm, H, Dh) * Dm ** (-0.5)), 'Wk': _w((lambda *s: _rng.normal(s) * 0.05)(Dm, H, Dh) * Dm ** (-0.5)), 'Wv': _w((lambda *s: _rng.normal(s) * 0.05)(Dm, H, Dh) * Dm ** (-0.5)), 'Wo': _w((lambda *s: _rng.normal(s) * 0.05)(H, Dh, Dm) * (H * Dh) ** (-0.5)), 'seg_len': seg}
    _A_in = _A_setup()

    def _B_setup():
        B, S, D, F = (1, 2048, 1024, 3584)
        return {'x': _w((lambda *s: _rng.normal(s) * 0.05)(B, S, D)), 'w1': _w((lambda *s: _rng.normal(s) * 0.05)(D, D) * D ** (-0.5)), 'w2': _w((lambda *s: _rng.normal(s) * 0.05)(D, D) * D ** (-0.5)), 'w3': _w((lambda *s: _rng.normal(s) * 0.05)(D, F) * D ** (-0.5)), 'w4': _w((lambda *s: _rng.normal(s) * 0.05)(F, D) * F ** (-0.5))}
    _B_in = _B_setup()
    return {'A_x': _A_in['x'], 'A_mem0': _A_in['mem0'], 'A_Wq': _A_in['Wq'], 'A_Wk': _A_in['Wk'], 'A_Wv': _A_in['Wv'], 'A_Wo': _A_in['Wo'], 'A_seg_len': _A_in['seg_len'], 'B_x': _B_in['x'], 'B_w1': _B_in['w1'], 'B_w2': _B_in['w2'], 'B_w3': _B_in['w3'], 'B_w4': _B_in['w4']}

def reference(A_x, A_mem0, A_Wq, A_Wk, A_Wv, A_Wo, A_seg_len, B_x, B_w1, B_w2, B_w3, B_w4):

    def _A_ref(x, mem0, Wq, Wk, Wv, Wo, seg_len):
        B, S, Dm = x.shape
        H, Dh = (Wq.shape[1], Wq.shape[2])
        M = mem0.shape[1]
        scale = Dh ** (-0.5)
        n_seg = S // seg_len
        L = M + seg_len
        idx = jnp.arange(L)
        mask = (idx[:, None] < M) | (idx[:, None] >= idx[None, :])
        mem = mem0
        outs = []
        for s in range(n_seg):
            xs = x[:, s * seg_len:(s + 1) * seg_len, :].copy()
            h = jnp.concatenate([mem, xs], axis=1)
            q = jnp.einsum('btd,dhe->bhte', h, Wq)
            k = jnp.einsum('btd,dhe->bhte', h, Wk)
            v = jnp.einsum('btd,dhe->bhte', h, Wv)
            scores = jnp.einsum('bhqe,bhke->bhqk', q, k) * scale
            scores = jnp.where(mask[None, None], scores, -1000000000.0)
            p = _softmax(scores, axis=-1)
            o = jnp.einsum('bhqk,bhke->bhqe', p, v)
            o = jnp.einsum('bhte,hed->btd', o, Wo)
            mem = o[:, :M, :].copy()
            outs.append(o[:, M:, :])
        return jnp.concatenate(outs, axis=1)

    def _B_ref(x, w1, w2, w3, w4):
        B, S, D = x.shape
        h = _gelu(_layernorm(x, axis=-1) @ w1)
        c = D // 4
        g0 = jnp.pad(h[:, :, 0 * c:1 * c], ((0, 0), (1, 0), (0, 0)))[:, :S, :]
        g1 = jnp.pad(h[:, :, 1 * c:2 * c], ((0, 0), (0, 1), (0, 0)))[:, 1:, :]
        g2 = jnp.pad(h[:, :, 2 * c:3 * c], ((0, 0), (2, 0), (0, 0)))[:, :S, :]
        g3 = jnp.pad(h[:, :, 3 * c:], ((0, 0), (0, 2), (0, 0)))[:, 2:, :]
        hs = jnp.concatenate([g0, g1, g2, g3], axis=-1) @ w2
        x1 = x + hs
        h2 = _gelu(_layernorm(x1, axis=-1) @ w3) @ w4
        return x1 + h2
    x = A_x
    h = x + _A_ref(_layernorm(x, axis=-1), A_mem0, A_Wq, A_Wk, A_Wv, A_Wo, A_seg_len)
    h2 = h + _B_ref(_layernorm(h, axis=-1), B_w1, B_w2, B_w3, B_w4)
    return h2
```

```python
import functools

import jax
import jax.numpy as jnp
import numpy as np
from jax import lax
from jax.experimental import pallas as pl
from jax.experimental.pallas import tpu as pltpu

f32, bf16, u32 = jnp.float32, jnp.bfloat16, jnp.uint32

S, D, H, E, M, F = 2048, 1024, 32, 128, 8, 3584
LN_EPS = 1e-5
DCH = 128
NCH = D // DCH
NSLOT = 4
PAD = 8


def _dot(a, b):
  return lax.dot_general(a, b, (((1,), (0,)), ((), ())), preferred_element_type=f32)


def _dot_nt(a, b):
  return lax.dot_general(a, b, (((1,), (1,)), ((), ())), preferred_element_type=f32)


def _bf(w):
  return pltpu.bitcast(w, bf16)


def _ln(x):
  m = jnp.mean(x, axis=-1, keepdims=True)
  d = x - m
  v = jnp.mean(d * d, axis=-1, keepdims=True)
  return d * lax.rsqrt(v + LN_EPS)


def _gelu(x):
  c = np.float32(np.sqrt(2.0 / np.pi))
  inner = x * (c + (np.float32(c * 0.044715)) * (x * x))
  return (0.5 * x) * (1.0 + jnp.tanh(inner))


def _rows(i, n):
  if isinstance(i, int):
    return pl.ds(i, n)
  return pl.ds(pl.multiple_of(i, 8), n)


def _kernel(seg, x_hbm, mem0_ref, wq_hbm, wk_hbm, wv_hbm, wo_hbm, w1_hbm, w2_hbm,
            w3_hbm, w4_hbm, out_ref,
            xv, wqkv, wo, w1, w2, w3, w4, stage, membuf, xnbuf, obuf, abuf, ybuf,
            habuf, h1buf, x1buf, zbuf, gbuf, st_sem, sems):
  nseg = S // seg
  L = M + seg
  scale = np.float32(E ** -0.5)

  x_cp = pltpu.make_async_copy(x_hbm, xv, sems.at[0])
  x_cp.start()

  qkv_hbm = (wq_hbm, wk_hbm, wv_hbm)

  def stage_cp(m, c, slot):
    src = qkv_hbm[m].at[pl.ds(c * (DCH * H), DCH * H)]
    return pltpu.make_async_copy(src, stage.at[slot].bitcast(bf16), st_sem.at[slot])

  def strips(w_hbm, dst, sem):
    n = dst.shape[0]
    return [
        pltpu.make_async_copy(
            w_hbm.at[:, pl.ds(j * 128, 128)], dst.at[j].bitcast(bf16), sem)
        for j in range(n)
    ]

  wo_cp = strips(wo_hbm, wo, sems.at[1])
  w1_cp = strips(w1_hbm, w1, sems.at[2])
  w2_cp = strips(w2_hbm, w2, sems.at[3])
  w3_cp = strips(w3_hbm, w3, sems.at[4])
  w4_cp = strips(w4_hbm, w4, sems.at[5])

  ahead = NSLOT - 1
  for c in range(ahead):
    stage_cp(0, c, c).start()

  h1buf[0:PAD, :] = jnp.zeros((PAD, D), f32)
  h1buf[PAD + S:PAD + S + PAD, :] = jnp.zeros((PAD, D), f32)
  membuf[...] = mem0_ref[...].astype(f32)

  for m in range(3):
    def relayout(c, _, m=m):
      slot = (m * NCH + c) % NSLOT
      nslot = (m * NCH + c + ahead) % NSLOT

      @pl.when(c + ahead < NCH)
      def _():
        stage_cp(m, c + ahead, nslot).start()

      if m < 2:
        @pl.when(c + ahead >= NCH)
        def _():
          stage_cp(m + 1, c + ahead - NCH, nslot).start()

      stage_cp(m, c, slot).wait()
      v = _bf(stage[slot]).reshape(DCH, H, E)
      t = jnp.swapaxes(v, 0, 1)
      r = pl.ds(pl.multiple_of(c * (DCH // 2), 8), DCH // 2)
      for h in range(H):
        wqkv[m * H + h, r, :] = pltpu.bitcast(t[h], u32)
      return 0

    lax.fori_loop(0, NCH, relayout, 0)

  for group in (wo_cp, w1_cp, w2_cp, w3_cp, w4_cp):
    for cp in group:
      cp.start()

  row = lax.broadcasted_iota(jnp.int32, (L, L), 0)
  col = lax.broadcasted_iota(jnp.int32, (L, L), 1)
  mask = (row < M) | (col <= row)

  def st_xn(s):
    xs = xv[_rows(s * seg, seg), :].astype(f32)
    xnbuf[s % 2] = _ln(xs)

  def st_qkv(s, h, m):
    lhs = jnp.concatenate([membuf[...], xnbuf[s % 2]], axis=0)
    return _dot(lhs, _bf(wqkv[m * H + h]))

  def st_scores(q, k):
    return _dot_nt(q, k.astype(bf16))

  def st_softmax(sc):
    sc = jnp.where(mask, sc * scale, np.float32(-1e9))
    mx = jnp.max(sc, axis=-1, keepdims=True)
    e = jnp.exp(sc - mx)
    l = jnp.sum(e, axis=-1, keepdims=True)
    return e, l

  def st_pv(h, e, l, v):
    o = _dot(e, v.astype(bf16))
    obuf[:, h * E:(h + 1) * E] = o * (1.0 / l)

  def st_wo(s, j):
    r = _dot(obuf[...], _bf(wo[j]))
    membuf[:, j * 128:(j + 1) * 128] = r[:M]
    abuf[:, j * 128:(j + 1) * 128] = r[M:]

  def st_post(t):
    xs = xv[_rows(t * seg, seg), :].astype(f32)
    ha = xs + abuf[...]
    habuf[t % 4] = ha
    y = _ln(ha)
    ybuf[t % 4] = y
    zbuf[0] = _ln(y)

  def st_b1(t, j):
    g = _gelu(_dot(zbuf[0], _bf(w1[j])))
    h1buf[_rows(PAD + t * seg, seg), j * 128:(j + 1) * 128] = g

  c4 = D // 4

  def st_shift(t):
    win = h1buf[_rows(t * seg, seg + 2 * PAD), :]
    g0 = win[PAD - 1:PAD - 1 + seg, 0 * c4:1 * c4]
    g1 = win[PAD + 1:PAD + 1 + seg, 1 * c4:2 * c4]
    g2 = win[PAD - 2:PAD - 2 + seg, 2 * c4:3 * c4]
    g3 = win[PAD + 2:PAD + 2 + seg, 3 * c4:4 * c4]
    zbuf[1] = jnp.concatenate([g0, g1, g2, g3], axis=1)

  def st_b2(t, j):
    cs = slice(j * 128, (j + 1) * 128)
    x1buf[:, cs] = ybuf[t % 4, :, cs] + _dot(zbuf[1], _bf(w2[j]))

  def st_ln2(t):
    zbuf[2] = _ln(x1buf[...])

  def st_b3(t, j):
    gbuf[:, j * 128:(j + 1) * 128] = _gelu(_dot(zbuf[2], _bf(w3[j])))

  def st_b4(t, j):
    cs = slice(j * 128, (j + 1) * 128)
    h2 = _dot(gbuf[...], _bf(w4[j]))
    res = habuf[t % 4, :, cs] + (x1buf[:, cs] + h2)
    out_ref[_rows(t * seg, seg), cs] = res.astype(out_ref.dtype)

  def step(s, do_r, do_b1, do_b2, waits=()):
    waits = dict(waits)
    fill = []
    t1, t2 = s - 1, s - 2
    nf3 = F // 128
    if do_b1:
      st_post(t1)
      fill.append(("w1", lambda: [st_b1(t1, j) for j in range(8)]))
    if do_b2:
      def b2():
        st_shift(t2)
        for j in range(8):
          st_b2(t2, j)
        st_ln2(t2)
      fill.append(("w2", b2))
      fill.append(("w3", lambda: [st_b3(t2, j) for j in range(0, nf3 // 2)]))
      fill.append((None, lambda: [st_b3(t2, j) for j in range(nf3 // 2, nf3)]))
      fill.append(("w4", lambda: [st_b4(t2, j) for j in range(0, 3)]))
      fill.append((None, lambda: [st_b4(t2, j) for j in range(3, 6)]))
      fill.append((None, lambda: [st_b4(t2, j) for j in range(6, 8)]))

    def run_fill():
      if fill:
        name, thunk = fill.pop(0)
        if name in waits:
          for cp in waits[name]:
            cp.wait()
        thunk()

    if do_r:
      if isinstance(s, int):
        if s + 1 < nseg:
          st_xn(s + 1)
      else:
        st_xn(jnp.minimum(s + 1, nseg - 1))
      qkv = {}
      sc = {}
      el = {}
      LAG_S, LAG_PV = 2, 4
      fill_after = {3: 1, 7: 1, 11: 1, 15: 1, 19: 1}

      def attn(h):
        hs, hp = h - LAG_S, h - LAG_PV
        if 0 <= hs < H:
          sc[hs] = st_scores(qkv[hs][0], qkv[hs][1])
        if 0 <= hp < H:
          e, l = st_softmax(sc.pop(hp))
          st_pv(hp, e, l, qkv.pop(hp)[2])

      for h in range(H):
        qkv[h] = [st_qkv(s, h, m) for m in range(3)]
        attn(h)
        if h in fill_after:
          run_fill()
      for h in range(H, H + LAG_PV):
        if h in (H, H + 2):
          run_fill()
        attn(h)
      if "wo" in waits:
        for cp in waits["wo"]:
          cp.wait()
      for j in range(8):
        st_wo(s, j)
    while fill:
      run_fill()

  x_cp.wait()
  st_xn(0)
  step(0, True, False, False, waits={"wo": wo_cp})
  step(1, True, True, False, waits={"w1": w1_cp})
  step(2, True, True, True, waits={"w2": w2_cp, "w3": w3_cp, "w4": w4_cp})

  def body(s, _):
    step(s, True, True, True)
    return 0

  lax.fori_loop(3, nseg, body, 0)
  step(nseg, False, True, True)
  step(nseg + 1, False, False, True)


def _forward(A_x, A_mem0, A_Wq, A_Wk, A_Wv, A_Wo, seg, B_w1, B_w2, B_w3, B_w4):
  assert A_x.shape == (1, S, D) and A_mem0.shape == (1, M, D)
  assert A_Wq.shape == (D, H, E) and A_Wo.shape == (H, E, D) and B_w3.shape == (D, F)
  assert seg == 32
  x2 = A_x.reshape(S, D)
  mem0 = A_mem0.reshape(M, D)
  wq, wk, wv = (w.reshape(D * H, E) for w in (A_Wq, A_Wk, A_Wv))
  wo = A_Wo.reshape(H * E, D)
  any_spec = pl.BlockSpec(memory_space=pl.ANY)
  scratch = [
      pltpu.VMEM((S, D), bf16),
      pltpu.VMEM((3 * H, D // 2, E), u32),
      pltpu.VMEM((D // 128, H * E // 2, 128), u32),
      pltpu.VMEM((D // 128, D // 2, 128), u32),
      pltpu.VMEM((D // 128, D // 2, 128), u32),
      pltpu.VMEM((F // 128, D // 2, 128), u32),
      pltpu.VMEM((D // 128, F // 2, 128), u32),
      pltpu.VMEM((NSLOT, DCH * H // 2, E), u32),
      pltpu.VMEM((M, D), f32),
      pltpu.VMEM((2, seg, D), f32),
      pltpu.VMEM((M + seg, H * E), f32),
      pltpu.VMEM((seg, D), f32),
      pltpu.VMEM((4, seg, D), f32),
      pltpu.VMEM((4, seg, D), f32),
      pltpu.VMEM((S + 2 * PAD, D), f32),
      pltpu.VMEM((seg, D), f32),
      pltpu.VMEM((3, seg, D), f32),
      pltpu.VMEM((seg, F), f32),
      pltpu.SemaphoreType.DMA((NSLOT,)),
      pltpu.SemaphoreType.DMA((6,)),
  ]
  out = pl.pallas_call(
      functools.partial(_kernel, seg),
      out_shape=jax.ShapeDtypeStruct((S, D), A_x.dtype),
      in_specs=[any_spec, pl.BlockSpec(memory_space=pltpu.VMEM)] + [any_spec] * 8,
      out_specs=pl.BlockSpec(memory_space=pltpu.VMEM),
      scratch_shapes=scratch,
      compiler_params=pltpu.CompilerParams(vmem_limit_bytes=110 * 2**20),
  )(x2, mem0, wq, wk, wv, wo, B_w1, B_w2, B_w3, B_w4)
  return out.reshape(1, S, D)


def pallas_sequential_preLN__memory_aug_recurrent_mem_tr__mixer_s_mlp__prompt_kernel(
    A_x, A_mem0, A_Wq, A_Wk, A_Wv, A_Wo, A_seg_len, B_x, B_w1, B_w2, B_w3, B_w4):
  del B_x
  return _forward(A_x, A_mem0, A_Wq, A_Wk, A_Wv, A_Wo, int(A_seg_len),
                  B_w1, B_w2, B_w3, B_w4)
```

```python
import functools

import jax
import jax.numpy as jnp
import numpy as np
from jax import lax
from jax.experimental import pallas as pl
from jax.experimental.pallas import tpu as pltpu

f32, bf16, u32 = jnp.float32, jnp.bfloat16, jnp.uint32

S, D, H, E, M, F = 2048, 1024, 32, 128, 8, 3584
LN_EPS = 1e-5
DCH = 128
NCH = D // DCH
NSLOT = 6
PAD = 8
XP = 512
RX = 24
RING = 768
RING0 = 64


def _dot(a, b):
  return lax.dot_general(a, b, (((1,), (0,)), ((), ())), preferred_element_type=f32)


def _dot_nt(a, b):
  return lax.dot_general(a, b, (((1,), (1,)), ((), ())), preferred_element_type=f32)


def _bf(w):
  return pltpu.bitcast(w, bf16)


def _ln(x):
  m = jnp.mean(x, axis=-1, keepdims=True)
  d = x - m
  v = jnp.mean(d * d, axis=-1, keepdims=True)
  return d * lax.rsqrt(v + LN_EPS)


def _gelu(x):
  c = np.float32(np.sqrt(2.0 / np.pi))
  inner = x * (c + (np.float32(c * 0.044715)) * (x * x))
  return (0.5 * x) * (1.0 + jnp.tanh(inner))


def _rows(i, n):
  if isinstance(i, int):
    return pl.ds(i, n)
  return pl.ds(pl.multiple_of(i, 8), n)


def _kernel(seg, x_hbm, mem0_ref, wq_hbm, wk_hbm, wv_hbm, wo_hbm, w1_hbm, w2_hbm,
            w3_hbm, w4_hbm, out_hbm,
            xv, wqkv, wo, w1, w2, w3, w4, stage, tba, tbb, xnp, qkvbuf, membuf, xnbuf,
            obuf, abuf, ybuf, habuf, h1buf, x1buf, zbuf, gbuf, outv, st_sem, sems):
  nseg = S // seg
  L = M + seg
  scale = np.float32(E ** -0.5)

  xa_cp = pltpu.make_async_copy(x_hbm.at[0:XP], xv.at[0:XP], sems.at[0])
  xb_cp = pltpu.make_async_copy(x_hbm.at[XP:S], xv.at[XP:S], sems.at[6])
  qkv_hbm = (wq_hbm, wk_hbm, wv_hbm)

  def stage_cp(m, c, slot):
    src = qkv_hbm[m].at[pl.ds(c * (DCH * H), DCH * H)]
    return pltpu.make_async_copy(src, stage.at[slot].bitcast(bf16), st_sem.at[slot])

  def stage_wait(g):
    stage_cp(0, 0, g % NSLOT).wait()

  def stage_start(g):
    for m in range(3):
      if isinstance(g, int):
        if m * NCH <= g < (m + 1) * NCH:
          stage_cp(m, g - m * NCH, g % NSLOT).start()
      else:
        @pl.when((g >= m * NCH) & (g < (m + 1) * NCH))
        def _(m=m):
          stage_cp(m, g - m * NCH, g % NSLOT).start()

  def strips(w_hbm, dst, sem):
    n = dst.shape[0]
    return [
        pltpu.make_async_copy(
            w_hbm.at[:, pl.ds(j * 128, 128)], dst.at[j].bitcast(bf16), sem)
        for j in range(n)
    ]

  wo_cp = strips(wo_hbm, wo, sems.at[1])
  w1_cp = strips(w1_hbm, w1, sems.at[2])
  w2_cp = strips(w2_hbm, w2, sems.at[3])
  w3_cp = strips(w3_hbm, w3, sems.at[4])
  w4_cp = strips(w4_hbm, w4, sems.at[5])

  xa_cp.start()
  for g in range(NSLOT - 1):
    stage_start(g)

  h1buf[0:PAD, :] = jnp.zeros((PAD, D), f32)
  h1buf[PAD + S:PAD + S + PAD, :] = jnp.zeros((PAD, D), f32)
  membuf[...] = mem0_ref[...].astype(f32)

  xa_cp.wait()
  LNB = 64

  def ln_pro(i, _):
    r = pl.ds(pl.multiple_of(i * LNB, LNB), LNB)
    xn = _ln(xv[r, :].astype(f32))
    for kc in range(NCH):
      xnp[kc, r, :] = xn[:, kc * 128:(kc + 1) * 128]
    return 0

  lax.fori_loop(0, XP // LNB, ln_pro, 0)

  def relayout(g, tb):
    v = _bf(stage[g % NSLOT]).reshape(DCH, H, E)
    t = jnp.swapaxes(v, 0, 1)
    m, kc = g // NCH, g % NCH
    r = _rows(kc * (DCH // 2), DCH // 2)
    for h in range(H):
      w = pltpu.bitcast(t[h], u32)
      tb[h] = w
      wqkv[m * H + h, r, :] = w

  def pro_dots(g, tb, may_be_first):
    m, kc = g // NCH, g % NCH
    for h in range(H):
      part = _dot(xnp[kc], _bf(tb[h]))
      dst = qkvbuf[h].at[m]
      old = dst[RING0:RING0 + XP, :]
      if may_be_first:
        old = jnp.where(kc == 0, np.float32(0), old)
      dst[RING0:RING0 + XP, :] = old + part

  NG = 3 * NCH
  others = wo_cp + w1_cp + w2_cp + w3_cp + w4_cp
  other_batches = [
      [xb_cp], wo_cp[0:2], wo_cp[2:4], wo_cp[4:6], wo_cp[6:8], w1_cp[0:5],
      w1_cp[5:8] + w2_cp[0:2], w2_cp[2:8], w3_cp[0:6], w3_cp[6:12], w3_cp[12:18]]
  tail_batch = w3_cp[18:28] + w4_cp
  del others

  stage_wait(0)
  relayout(0, tba)

  def pro_body(i, _):
    g = 2 * i
    stage_start(g + NSLOT - 1)
    stage_start(g + NSLOT)
    for b, batch in enumerate(other_batches):
      @pl.when(i == b)
      def _(batch=batch):
        for cp in batch:
          cp.start()
    stage_wait(g + 1)
    stage_wait(g + 2)
    relayout(g + 1, tbb)
    pro_dots(g, tba, True)
    relayout(g + 2, tba)
    pro_dots(g + 1, tbb, False)
    return 0

  lax.fori_loop(0, NG // 2 - 1, pro_body, 0)
  for batch in other_batches[NG // 2 - 1:]:
    for cp in batch:
      cp.start()
  for cp in tail_batch:
    cp.start()
  stage_wait(NG - 1)
  relayout(NG - 1, tbb)
  pro_dots(NG - 2, tba, False)
  pro_dots(NG - 1, tbb, False)

  row = lax.broadcasted_iota(jnp.int32, (L, L), 0)
  col = lax.broadcasted_iota(jnp.int32, (L, L), 1)
  mask = (row < M) | (col <= row)

  def st_xn(s):
    xs = xv[_rows(XP + s * RX, RX), :].astype(f32)
    xnbuf[s % 2] = _ln(xs)

  def wrow(s):
    return _rows(((s + (XP + RING0) // RX) % (RING // RX)) * RX, RX)

  def rrow(s):
    return _rows(((s + RING0 // seg) % (RING // seg)) * seg, seg)

  def st_qkv(s, h, m):
    lhs = jnp.concatenate([membuf[...], xnbuf[s % 2]], axis=0)
    r = _dot(lhs, _bf(wqkv[m * H + h]))
    qkvbuf[h][m, wrow(s), :] = r[M:]
    return r[:M]

  def ld(s, h, m, fresh):
    return jnp.concatenate([fresh, qkvbuf[h][m, rrow(s), :]], axis=0)

  def st_scores(q, k):
    return _dot_nt(q, k.astype(bf16))

  def st_softmax(sc):
    sc = jnp.where(mask, sc * scale, np.float32(-1e9))
    mx = jnp.max(sc, axis=-1, keepdims=True)
    e = jnp.exp(sc - mx)
    l = jnp.sum(e, axis=-1, keepdims=True)
    return e, l

  def st_pv(h, e, l, v):
    o = _dot(e, v.astype(bf16))
    obuf[:, h * E:(h + 1) * E] = o * (1.0 / l)

  def st_wo(s, j):
    r = _dot(obuf[...], _bf(wo[j]))
    membuf[:, j * 128:(j + 1) * 128] = r[:M]
    abuf[:, j * 128:(j + 1) * 128] = r[M:]

  def st_post(t):
    xs = xv[_rows(t * seg, seg), :].astype(f32)
    ha = xs + abuf[...]
    habuf[t % 4] = ha
    y = _ln(ha)
    ybuf[t % 4] = y
    zbuf[0] = _ln(y)

  def st_b1(t, j):
    g = _gelu(_dot(zbuf[0], _bf(w1[j])))
    h1buf[_rows(PAD + t * seg, seg), j * 128:(j + 1) * 128] = g

  c4 = D // 4

  def st_shift(t):
    win = h1buf[_rows(t * seg, seg + 2 * PAD), :]
    g0 = win[PAD - 1:PAD - 1 + seg, 0 * c4:1 * c4]
    g1 = win[PAD + 1:PAD + 1 + seg, 1 * c4:2 * c4]
    g2 = win[PAD - 2:PAD - 2 + seg, 2 * c4:3 * c4]
    g3 = win[PAD + 2:PAD + 2 + seg, 3 * c4:4 * c4]
    zbuf[1] = jnp.concatenate([g0, g1, g2, g3], axis=1)

  def st_b2(t, j):
    cs = slice(j * 128, (j + 1) * 128)
    x1buf[:, cs] = ybuf[t % 4, :, cs] + _dot(zbuf[1], _bf(w2[j]))

  def st_ln2(t):
    zbuf[2] = _ln(x1buf[...])

  def st_b3(t, j):
    gbuf[:, j * 128:(j + 1) * 128] = _gelu(_dot(zbuf[2], _bf(w3[j])))

  def st_b4(t, j):
    cs = slice(j * 128, (j + 1) * 128)
    h2 = _dot(gbuf[...], _bf(w4[j]))
    res = habuf[t % 4, :, cs] + (x1buf[:, cs] + h2)
    outv[_rows(t * seg, seg), cs] = res.astype(outv.dtype)

  def st_out(t):
    r = _rows(t * seg, seg)
    pltpu.make_async_copy(outv.at[r], out_hbm.at[r], sems.at[7]).start()

  def step(s, do_r, do_b1, do_b2, waits=()):
    waits = dict(waits)
    fill = []
    t1, t2 = s - 1, s - 2
    nf3 = F // 128
    if do_b1:
      st_post(t1)
      fill.append(("w1", lambda: [st_b1(t1, j) for j in range(8)]))
    if do_b2:
      def b2():
        st_shift(t2)
        for j in range(8):
          st_b2(t2, j)
        st_ln2(t2)

      def b4_last():
        for j in range(6, 8):
          st_b4(t2, j)
        st_out(t2)

      fill.append(("w2", b2))
      fill.append(("w3", lambda: [st_b3(t2, j) for j in range(0, nf3 // 2)]))
      fill.append((None, lambda: [st_b3(t2, j) for j in range(nf3 // 2, nf3)]))
      fill.append(("w4", lambda: [st_b4(t2, j) for j in range(0, 3)]))
      fill.append((None, lambda: [st_b4(t2, j) for j in range(3, 6)]))
      fill.append((None, b4_last))

    def run_fill():
      if fill:
        name, thunk = fill.pop(0)
        if name in waits:
          for cp in waits[name]:
            cp.wait()
        thunk()

    if do_r:
      if "xb" in waits:
        waits["xb"].wait()
      fresh = {}
      sc = {}
      LAG_S, LAG_PV = 2, 4
      fill_after = {3: 1, 7: 1, 11: 1, 15: 1, 19: 1}

      def attn(h):
        hs, hp = h - LAG_S, h - LAG_PV
        if 0 <= hs < H:
          sc[hs] = st_scores(ld(s, hs, 0, fresh[hs][0]), ld(s, hs, 1, fresh[hs][1]))
        if 0 <= hp < H:
          e, l = st_softmax(sc.pop(hp))
          st_pv(hp, e, l, ld(s, hp, 2, fresh.pop(hp)[2]))

      for h in range(H):
        fresh[h] = [st_qkv(s, h, m) for m in range(3)]
        attn(h)
        if h in fill_after:
          run_fill()
      for h in range(H, H + LAG_PV):
        if h in (H, H + 2):
          run_fill()
        attn(h)
      if isinstance(s, int):
        if s + 1 < nseg:
          st_xn(s + 1)
      else:
        st_xn(jnp.minimum(s + 1, nseg - 1))
      if "wo" in waits:
        for cp in waits["wo"]:
          cp.wait()
      for j in range(8):
        st_wo(s, j)
    while fill:
      run_fill()

  xb_cp.wait()
  st_xn(0)
  step(0, True, False, False, waits={"wo": wo_cp})
  step(1, True, True, False, waits={"w1": w1_cp})
  step(2, True, True, True, waits={"w2": w2_cp, "w3": w3_cp, "w4": w4_cp})

  def body(s, _):
    step(s, True, True, True)
    return 0

  lax.fori_loop(3, nseg, body, 0)
  step(nseg, False, True, True)
  step(nseg + 1, False, False, True)
  pltpu.make_async_copy(outv, out_hbm, sems.at[7]).wait()


def _forward(A_x, A_mem0, A_Wq, A_Wk, A_Wv, A_Wo, seg, B_w1, B_w2, B_w3, B_w4):
  assert A_x.shape == (1, S, D) and A_mem0.shape == (1, M, D)
  assert A_Wq.shape == (D, H, E) and A_Wo.shape == (H, E, D) and B_w3.shape == (D, F)
  assert seg == 32 and XP + (S // seg) * RX == S
  x2 = A_x.reshape(S, D)
  mem0 = A_mem0.reshape(M, D)
  wq, wk, wv = (w.reshape(D * H, E) for w in (A_Wq, A_Wk, A_Wv))
  wo = A_Wo.reshape(H * E, D)
  any_spec = pl.BlockSpec(memory_space=pl.ANY)
  scratch = [
      pltpu.VMEM((S, D), bf16),
      pltpu.VMEM((3 * H, D // 2, E), u32),
      pltpu.VMEM((D // 128, H * E // 2, 128), u32),
      pltpu.VMEM((D // 128, D // 2, 128), u32),
      pltpu.VMEM((D // 128, D // 2, 128), u32),
      pltpu.VMEM((F // 128, D // 2, 128), u32),
      pltpu.VMEM((D // 128, F // 2, 128), u32),
      pltpu.VMEM((NSLOT, DCH * H // 2, E), u32),
      pltpu.VMEM((H, DCH // 2, E), u32),
      pltpu.VMEM((H, DCH // 2, E), u32),
      pltpu.VMEM((NCH, XP, 128), f32),
      [pltpu.VMEM((3, RING, E), f32) for _ in range(H)],
      pltpu.VMEM((M, D), f32),
      pltpu.VMEM((2, RX, D), f32),
      pltpu.VMEM((M + seg, H * E), f32),
      pltpu.VMEM((seg, D), f32),
      pltpu.VMEM((4, seg, D), f32),
      pltpu.VMEM((4, seg, D), f32),
      pltpu.VMEM((S + 2 * PAD, D), f32),
      pltpu.VMEM((seg, D), f32),
      pltpu.VMEM((3, seg, D), f32),
      pltpu.VMEM((seg, F), f32),
      pltpu.VMEM((S, D), A_x.dtype),
      pltpu.SemaphoreType.DMA((NSLOT,)),
      pltpu.SemaphoreType.DMA((8,)),
  ]
  out = pl.pallas_call(
      functools.partial(_kernel, seg),
      out_shape=jax.ShapeDtypeStruct((S, D), A_x.dtype),
      in_specs=[any_spec, pl.BlockSpec(memory_space=pltpu.VMEM)] + [any_spec] * 8,
      out_specs=any_spec,
      scratch_shapes=scratch,
      compiler_params=pltpu.CompilerParams(vmem_limit_bytes=126 * 2**20),
  )(x2, mem0, wq, wk, wv, wo, B_w1, B_w2, B_w3, B_w4)
  return out.reshape(1, S, D)


def pallas_sequential_preLN__memory_aug_recurrent_mem_tr__mixer_s_mlp__prompt_kernel(
    A_x, A_mem0, A_Wq, A_Wk, A_Wv, A_Wo, A_seg_len, B_x, B_w1, B_w2, B_w3, B_w4):
  del B_x
  return _forward(A_x, A_mem0, A_Wq, A_Wk, A_Wv, A_Wo, int(A_seg_len),
                  B_w1, B_w2, B_w3, B_w4)
```

```python
import functools

import jax
import jax.numpy as jnp
import numpy as np
from jax import lax
from jax.experimental import pallas as pl
from jax.experimental.pallas import tpu as pltpu

f32, bf16, u32 = jnp.float32, jnp.bfloat16, jnp.uint32

S, D, H, E, M, F = 2048, 1024, 32, 128, 8, 3584
LN_EPS = 1e-5
LOG2E = float(np.log2(np.e))
DCH = 128
NCH = D // DCH
NSLOT = 6
PAD = 8
XP = 512
RX = 24
RING = 768
UNROLL = 1
HG = 4
SCHEDULE = """
    POST Q0 Q1 S0 B1 Q2 S1 P0 B2 Q3 S2 P1 B3a Q4 S3 P2 B3b Q5 S4 P3 Q6 S5 P4 B4a
    Q7 S6 P5 XN B4b S7 P6 B4c P7 WO
"""
RING0 = 64


def _dot(a, b):
  return lax.dot_general(a, b, (((1,), (0,)), ((), ())), preferred_element_type=f32)


def _dot_nt(a, b):
  return lax.dot_general(a, b, (((1,), (1,)), ((), ())), preferred_element_type=f32)


def _bf(w):
  return pltpu.bitcast(w, bf16)


def _pk(x):
  return pltpu.bitcast(x.astype(bf16), u32)


def _ln(x):
  m = jnp.mean(x, axis=-1, keepdims=True)
  d = x - m
  v = jnp.mean(d * d, axis=-1, keepdims=True)
  return d * lax.rsqrt(v + LN_EPS)


def _gelu(x):
  c = np.float32(np.sqrt(2.0 / np.pi))
  inner = x * (c + (np.float32(c * 0.044715)) * (x * x))
  return (0.5 * x) * (1.0 + jnp.tanh(inner))


def _rows(i, n):
  if isinstance(i, int):
    return pl.ds(i, n)
  return pl.ds(pl.multiple_of(i, 8), n)


def _kernel(seg, x_hbm, mem0_ref, wq_hbm, wk_hbm, wv_hbm, wo_hbm, w1_hbm, w2_hbm,
            w3_hbm, w4_hbm, out_hbm,
            xv, wqkv, wo, w1, w2, w3, w4, stage, tba, tbb, xnp, qkvbuf, membuf, xnbuf,
            obuf, abuf, ybuf, habuf, h1buf, x1buf, zbuf, gbuf, outv, st_sem, sems):
  nseg = S // seg
  L = M + seg
  scale = np.float32(E ** -0.5)

  xa_cp = pltpu.make_async_copy(x_hbm.at[0:XP], xv.at[0:XP], sems.at[0])
  xb_cp = pltpu.make_async_copy(x_hbm.at[XP:S], xv.at[XP:S], sems.at[6])
  qkv_hbm = (wq_hbm, wk_hbm, wv_hbm)

  def stage_cp(m, c, slot):
    src = qkv_hbm[m].at[pl.ds(c * (DCH * H), DCH * H)]
    return pltpu.make_async_copy(src, stage.at[slot].bitcast(bf16), st_sem.at[slot])

  def stage_wait(g):
    stage_cp(0, 0, g % NSLOT).wait()

  def stage_start(g):
    for m in range(3):
      if isinstance(g, int):
        if m * NCH <= g < (m + 1) * NCH:
          stage_cp(m, g - m * NCH, g % NSLOT).start()
      else:
        @pl.when((g >= m * NCH) & (g < (m + 1) * NCH))
        def _(m=m):
          stage_cp(m, g - m * NCH, g % NSLOT).start()

  def strips(w_hbm, dst, sem):
    n = dst.shape[0]
    return [
        pltpu.make_async_copy(
            w_hbm.at[:, pl.ds(j * 128, 128)], dst.at[j].bitcast(bf16), sem)
        for j in range(n)
    ]

  wo_cp = strips(wo_hbm, wo, sems.at[1])
  w1_cp = strips(w1_hbm, w1, sems.at[2])
  w2_cp = strips(w2_hbm, w2, sems.at[3])
  w3_cp = strips(w3_hbm, w3, sems.at[4])
  w4_cp = strips(w4_hbm, w4, sems.at[5])

  xa_cp.start()
  for g in range(NSLOT - 1):
    stage_start(g)

  h1buf[0:PAD, :] = jnp.zeros((PAD, D), f32)
  h1buf[PAD + S:PAD + S + PAD, :] = jnp.zeros((PAD, D), f32)
  membuf[...] = mem0_ref[...].astype(f32)

  xa_cp.wait()
  LNB = 64

  def ln_pro(i, _):
    r = pl.ds(pl.multiple_of(i * LNB, LNB), LNB)
    xn = _ln(xv[r, :].astype(f32))
    for kc in range(NCH):
      xnp[kc, r, :] = xn[:, kc * 128:(kc + 1) * 128]
    return 0

  lax.fori_loop(0, XP // LNB, ln_pro, 0)

  def relayout(g, tb):
    v = _bf(stage[g % NSLOT]).reshape(DCH, H, E)
    t = jnp.swapaxes(v, 0, 1)
    m, kc = g // NCH, g % NCH
    r = _rows(kc * (DCH // 2), DCH // 2)
    for h in range(H):
      w = pltpu.bitcast(t[h], u32)
      tb[h] = w
      wqkv[m * H + h, r, :] = w

  def pro_dots(g, tb, may_be_first):
    m, kc = g // NCH, g % NCH
    for h in range(H):
      part = _dot(xnp[kc], _bf(tb[h]))
      dst = qkvbuf[h].at[m]
      old = dst[RING0:RING0 + XP, :]
      if may_be_first:
        old = jnp.where(kc == 0, np.float32(0), old)
      dst[RING0:RING0 + XP, :] = old + part

  NG = 3 * NCH
  others = wo_cp + w1_cp + w2_cp + w3_cp + w4_cp
  other_batches = [
      [xb_cp], wo_cp[0:2], wo_cp[2:4], wo_cp[4:6], wo_cp[6:8], w1_cp[0:5],
      w1_cp[5:8] + w2_cp[0:2], w2_cp[2:8], w3_cp[0:6], w3_cp[6:12], w3_cp[12:18]]
  tail_batch = w3_cp[18:28] + w4_cp
  del others

  stage_wait(0)
  relayout(0, tba)

  def pro_body(i, _):
    g = 2 * i
    stage_start(g + NSLOT - 1)
    stage_start(g + NSLOT)
    for b, batch in enumerate(other_batches):
      @pl.when(i == b)
      def _(batch=batch):
        for cp in batch:
          cp.start()
    stage_wait(g + 1)
    stage_wait(g + 2)
    relayout(g + 1, tbb)
    pro_dots(g, tba, True)
    relayout(g + 2, tba)
    pro_dots(g + 1, tbb, False)
    return 0

  lax.fori_loop(0, NG // 2 - 1, pro_body, 0)
  for batch in other_batches[NG // 2 - 1:]:
    for cp in batch:
      cp.start()
  for cp in tail_batch:
    cp.start()
  stage_wait(NG - 1)
  relayout(NG - 1, tbb)
  pro_dots(NG - 2, tba, False)
  pro_dots(NG - 1, tbb, False)

  row = lax.broadcasted_iota(jnp.int32, (L, L), 0)
  col = lax.broadcasted_iota(jnp.int32, (L, L), 1)
  mask = (row < M) | (col <= row)

  def st_xn(s):
    xs = xv[_rows(XP + s * RX, RX), :].astype(f32)
    xnbuf[s % 2] = _ln(xs)

  def wrow(s):
    return _rows(((s + (XP + RING0) // RX) % (RING // RX)) * RX, RX)

  def rrow(s):
    return _rows(((s + RING0 // seg) % (RING // seg)) * seg, seg)

  def st_lhs(s):
    return jnp.concatenate([membuf[...], xnbuf[s % 2]], axis=0).astype(bf16)

  def st_qkv(s, lhs, h, m):
    r = _dot(lhs, _bf(wqkv[m * H + h]))
    qkvbuf[h][m, wrow(s), :] = r[M:]
    return r[:M]

  def ld(s, h, m, fresh):
    return jnp.concatenate([fresh, qkvbuf[h][m, rrow(s), :]], axis=0)

  def st_scores(q, k):
    return _dot_nt(q, k.astype(bf16))

  def st_softmax(sc):
    t = jnp.where(mask, sc * np.float32(scale * LOG2E), np.float32(-1e9 * LOG2E))
    e = jnp.exp2(t - jnp.max(t, axis=-1, keepdims=True))
    l = jnp.sum(e, axis=-1, keepdims=True)
    r = pl.reciprocal(l, approx=True)
    r = r * (2.0 - l * r)
    return e * r

  def st_pv(h, p, v):
    obuf[:, h * E:(h + 1) * E] = _dot(p, v.astype(bf16))

  def st_wo(s, j):
    r = _dot(obuf[...], _bf(wo[j]))
    membuf[:, j * 128:(j + 1) * 128] = r[:M]
    abuf[:, j * 128:(j + 1) * 128] = r[M:]

  def st_post(t):
    xs = xv[_rows(t * seg, seg), :].astype(f32)
    ha = xs + abuf[...]
    habuf[t % 4] = ha
    y = _ln(ha)
    ybuf[t % 4] = y
    zbuf[0] = _pk(_ln(y))

  def st_b1(t, j):
    g = _gelu(_dot(_bf(zbuf[0]), _bf(w1[j])))
    h1buf[_rows(PAD + t * seg, seg), j * 128:(j + 1) * 128] = g

  c4 = D // 4

  def st_shift(t):
    win = h1buf[_rows(t * seg, seg + 2 * PAD), :]
    g0 = win[PAD - 1:PAD - 1 + seg, 0 * c4:1 * c4]
    g1 = win[PAD + 1:PAD + 1 + seg, 1 * c4:2 * c4]
    g2 = win[PAD - 2:PAD - 2 + seg, 2 * c4:3 * c4]
    g3 = win[PAD + 2:PAD + 2 + seg, 3 * c4:4 * c4]
    zbuf[1] = _pk(jnp.concatenate([g0, g1, g2, g3], axis=1))

  def st_b2(t, j):
    cs = slice(j * 128, (j + 1) * 128)
    x1buf[:, cs] = ybuf[t % 4, :, cs] + _dot(_bf(zbuf[1]), _bf(w2[j]))

  def st_ln2(t):
    zbuf[2] = _pk(_ln(x1buf[...]))

  def st_b3(t, j):
    gbuf[:, j * 128:(j + 1) * 128] = _pk(_gelu(_dot(_bf(zbuf[2]), _bf(w3[j]))))

  def st_b4(t, j):
    cs = slice(j * 128, (j + 1) * 128)
    h2 = _dot(_bf(gbuf[...]), _bf(w4[j]))
    res = habuf[t % 4, :, cs] + (x1buf[:, cs] + h2)
    outv[_rows(t * seg, seg), cs] = res.astype(outv.dtype)

  def st_out(t):
    r = _rows(t * seg, seg)
    pltpu.make_async_copy(outv.at[r], out_hbm.at[r], sems.at[7]).start()

  def step(s, do_r, do_b1, do_b2, waits=()):
    waits = dict(waits)
    t1, t2 = s - 1, s - 2
    nf3 = F // 128
    ops = {}

    def wait(name):
      for cp in waits.get(name, ()):
        cp.wait()

    if do_r:
      fresh, probs = {}, {}
      lhs = st_lhs(s)
      heads = lambda g: range(g * HG, (g + 1) * HG)

      def op_q(g):
        for h in heads(g):
          fresh[h] = [st_qkv(s, lhs, h, m) for m in range(3)]

      def op_s(g):
        sc = [st_scores(ld(s, h, 0, fresh[h][0]), ld(s, h, 1, fresh[h][1]))
              for h in heads(g)]
        for h, v in zip(heads(g), sc):
          probs[h] = st_softmax(v)

      def op_p(g):
        vs = [ld(s, h, 2, fresh.pop(h)[2]) for h in heads(g)]
        for h, v in zip(heads(g), vs):
          st_pv(h, probs.pop(h), v)

      def op_xn():
        if isinstance(s, int):
          if s + 1 < nseg:
            st_xn(s + 1)
        else:
          st_xn(jnp.minimum(s + 1, nseg - 1))

      def op_wo(js):
        if js[0] == 0:
          wait("wo")
        for j in js:
          st_wo(s, j)

      for g in range(H // HG):
        ops[f"Q{g}"] = functools.partial(op_q, g)
        ops[f"S{g}"] = functools.partial(op_s, g)
        ops[f"P{g}"] = functools.partial(op_p, g)
      ops["XN"] = op_xn
      ops["WO"] = lambda: op_wo(range(8))

    if do_b1:
      def op_b1():
        wait("w1")
        for j in range(8):
          st_b1(t1, j)
      ops["POST"] = lambda: st_post(t1)
      ops["B1"] = op_b1

    if do_b2:
      def op_b2():
        wait("w2")
        st_shift(t2)
        for j in range(8):
          st_b2(t2, j)
        st_ln2(t2)

      def op_b3(js):
        if js[0] == 0:
          wait("w3")
        for j in js:
          st_b3(t2, j)

      def op_b4(js):
        if js[0] == 0:
          wait("w4")
        for j in js:
          st_b4(t2, j)
        if js[-1] == 7:
          st_out(t2)

      ops["B2"] = op_b2
      ops["B3a"] = lambda: op_b3(range(0, nf3 // 2))
      ops["B3b"] = lambda: op_b3(range(nf3 // 2, nf3))
      ops["B4a"] = lambda: op_b4(range(0, 3))
      ops["B4b"] = lambda: op_b4(range(3, 6))
      ops["B4c"] = lambda: op_b4(range(6, 8))

    for name in SCHEDULE.split():
      if name in ops:
        ops.pop(name)()
    assert not ops, ops

  xb_cp.wait()
  st_xn(0)
  step(0, True, False, False, waits={"wo": wo_cp})
  step(1, True, True, False, waits={"w1": w1_cp})
  step(2, True, True, True, waits={"w2": w2_cp, "w3": w3_cp, "w4": w4_cp})

  first = 3 + (nseg - 3) % UNROLL
  for s in range(3, first):
    step(s, True, True, True)

  def body(i, _):
    for u in range(UNROLL):
      step(first + i * UNROLL + u, True, True, True)
    return 0

  lax.fori_loop(0, (nseg - first) // UNROLL, body, 0)
  step(nseg, False, True, True)
  step(nseg + 1, False, False, True)
  pltpu.make_async_copy(outv, out_hbm, sems.at[7]).wait()


def _forward(A_x, A_mem0, A_Wq, A_Wk, A_Wv, A_Wo, seg, B_w1, B_w2, B_w3, B_w4):
  assert A_x.shape == (1, S, D) and A_mem0.shape == (1, M, D)
  assert A_Wq.shape == (D, H, E) and A_Wo.shape == (H, E, D) and B_w3.shape == (D, F)
  assert seg == 32 and XP + (S // seg) * RX == S
  x2 = A_x.reshape(S, D)
  mem0 = A_mem0.reshape(M, D)
  wq, wk, wv = (w.reshape(D * H, E) for w in (A_Wq, A_Wk, A_Wv))
  wo = A_Wo.reshape(H * E, D)
  any_spec = pl.BlockSpec(memory_space=pl.ANY)
  scratch = [
      pltpu.VMEM((S, D), bf16),
      pltpu.VMEM((3 * H, D // 2, E), u32),
      pltpu.VMEM((D // 128, H * E // 2, 128), u32),
      pltpu.VMEM((D // 128, D // 2, 128), u32),
      pltpu.VMEM((D // 128, D // 2, 128), u32),
      pltpu.VMEM((F // 128, D // 2, 128), u32),
      pltpu.VMEM((D // 128, F // 2, 128), u32),
      pltpu.VMEM((NSLOT, DCH * H // 2, E), u32),
      pltpu.VMEM((H, DCH // 2, E), u32),
      pltpu.VMEM((H, DCH // 2, E), u32),
      pltpu.VMEM((NCH, XP, 128), f32),
      [pltpu.VMEM((3, RING, E), f32) for _ in range(H)],
      pltpu.VMEM((M, D), f32),
      pltpu.VMEM((2, RX, D), f32),
      pltpu.VMEM((M + seg, H * E), f32),
      pltpu.VMEM((seg, D), f32),
      pltpu.VMEM((4, seg, D), f32),
      pltpu.VMEM((4, seg, D), f32),
      pltpu.VMEM((S + 2 * PAD, D), f32),
      pltpu.VMEM((seg, D), f32),
      pltpu.VMEM((3, seg // 2, D), u32),
      pltpu.VMEM((seg // 2, F), u32),
      pltpu.VMEM((S, D), A_x.dtype),
      pltpu.SemaphoreType.DMA((NSLOT,)),
      pltpu.SemaphoreType.DMA((8,)),
  ]
  out = pl.pallas_call(
      functools.partial(_kernel, seg),
      out_shape=jax.ShapeDtypeStruct((S, D), A_x.dtype),
      in_specs=[any_spec, pl.BlockSpec(memory_space=pltpu.VMEM)] + [any_spec] * 8,
      out_specs=any_spec,
      scratch_shapes=scratch,
      compiler_params=pltpu.CompilerParams(vmem_limit_bytes=126 * 2**20),
  )(x2, mem0, wq, wk, wv, wo, B_w1, B_w2, B_w3, B_w4)
  return out.reshape(1, S, D)


def pallas_sequential_preLN__memory_aug_recurrent_mem_tr__mixer_s_mlp__prompt_kernel(
    A_x, A_mem0, A_Wq, A_Wk, A_Wv, A_Wo, A_seg_len, B_x, B_w1, B_w2, B_w3, B_w4):
  del B_x
  return _forward(A_x, A_mem0, A_Wq, A_Wk, A_Wv, A_Wo, int(A_seg_len),
                  B_w1, B_w2, B_w3, B_w4)
```

```python
import functools

import jax
import jax.numpy as jnp
import numpy as np
from jax import lax
from jax.experimental import pallas as pl
from jax.experimental.pallas import tpu as pltpu

f32, bf16, u32 = jnp.float32, jnp.bfloat16, jnp.uint32

S, D, H, E, M, F = 2048, 1024, 32, 128, 8, 3584
LN_EPS = 1e-5
LOG2E = float(np.log2(np.e))
DCH = 128
NCH = D // DCH
NSLOT = 6
PAD = 8
XP = 512
PRB = 128
RX = 24
RING = 768
UNROLL = 1
HG = 4
SCHEDULE = """
    POST Q0 Q1 S0 B1 Q2 S1 P0 B2 Q3 S2 P1 B3a Q4 S3 P2 B3b Q5 S4 P3 Q6 S5 P4 B4a
    Q7 S6 P5 XN B4b S7 P6 B4c P7 WO
"""
RING0 = 64


def _dot(a, b):
  return lax.dot_general(a, b, (((1,), (0,)), ((), ())), preferred_element_type=f32)


def _dot_nt(a, b):
  return lax.dot_general(a, b, (((1,), (1,)), ((), ())), preferred_element_type=f32)


def _bf(w):
  return pltpu.bitcast(w, bf16)


def _pk(x):
  return pltpu.bitcast(x.astype(bf16), u32)


def _ln(x):
  m = jnp.mean(x, axis=-1, keepdims=True)
  d = x - m
  v = jnp.mean(d * d, axis=-1, keepdims=True)
  return d * lax.rsqrt(v + LN_EPS)


def _gelu(x):
  c = np.float32(np.sqrt(2.0 / np.pi))
  inner = x * (c + (np.float32(c * 0.044715)) * (x * x))
  return (0.5 * x) * (1.0 + jnp.tanh(inner))


def _rows(i, n):
  if isinstance(i, int):
    return pl.ds(i, n)
  return pl.ds(pl.multiple_of(i, 8), n)


def _kernel(seg, x_hbm, mem0_ref, wq_hbm, wk_hbm, wv_hbm, wo_hbm, w1_hbm, w2_hbm,
            w3_hbm, w4_hbm, out_hbm,
            xv, wqa, wqb, wo, w1, w2, w3, w4, stage, xnp, qkvbuf, membuf, xnbuf,
            obuf, abuf, ybuf, habuf, h1buf, x1buf, zbuf, gbuf, outv, st_sem, sems):
  nseg = S // seg
  L = M + seg
  scale = np.float32(E ** -0.5)

  xa_cp = pltpu.make_async_copy(x_hbm.at[0:XP], xv.at[0:XP], sems.at[0])
  xb_cp = pltpu.make_async_copy(x_hbm.at[XP:S], xv.at[XP:S], sems.at[6])
  qkv_hbm = (wq_hbm, wk_hbm, wv_hbm)

  def stage_cp(m, c, slot):
    src = qkv_hbm[m].at[pl.ds(c * DCH, DCH)]
    return pltpu.make_async_copy(src, stage.at[slot].bitcast(bf16), st_sem.at[slot])

  def stage_wait(g):
    stage_cp(0, 0, g % NSLOT).wait()

  def stage_start(g):
    for m in range(3):
      if isinstance(g, int):
        if m * NCH <= g < (m + 1) * NCH:
          stage_cp(m, g - m * NCH, g % NSLOT).start()
      else:
        @pl.when((g >= m * NCH) & (g < (m + 1) * NCH))
        def _(m=m):
          stage_cp(m, g - m * NCH, g % NSLOT).start()

  strip_src = {"wo": (wo_hbm, wo, 1), "w1": (w1_hbm, w1, 2), "w2": (w2_hbm, w2, 3),
               "w3": (w3_hbm, w3, 4), "w4": (w4_hbm, w4, 5)}

  def strip(name, j):
    w_hbm, dst, sem = strip_src[name]
    col = j * 128 if isinstance(j, int) else pl.multiple_of(j * 128, 128)
    return pltpu.make_async_copy(
        w_hbm.at[:, pl.ds(col, 128)], dst.at[j].bitcast(bf16), sems.at[sem])

  def strips(name):
    return [strip(name, j) for j in range(strip_src[name][1].shape[0])]

  xa_cp.start()
  stage_start(0)
  h1buf[0:PAD, :] = jnp.zeros((PAD, D), f32)
  h1buf[PAD + S:PAD + S + PAD, :] = jnp.zeros((PAD, D), f32)
  membuf[...] = mem0_ref[...].astype(f32)

  xa_cp.wait()
  for g in range(1, NSLOT):
    stage_start(g)
  LNB = 64
  for i in range(XP // LNB):
    r = pl.ds(i * LNB, LNB)
    xn = _pk(_ln(xv[r, :].astype(f32)))
    for kc in range(NCH):
      xnp[kc, pl.ds(i * (LNB // 2), LNB // 2), :] = xn[:, kc * 128:(kc + 1) * 128]

  def _pk_rows(g, off, n):
    return _rows(((g % NCH) // 2) * (DCH // 2) + off, n)

  NU = 2 * DCH // 16

  def relayout(g, wdst, units=range(NU)):
    for u in units:
      db, p = u // 2, u % 2
      v = _bf(stage[g % NSLOT, pl.ds(db * 16, 16), pl.ds(p * 8, 8), :])
      t = jnp.swapaxes(v, 0, 1)
      for k in range(16):
        wdst[(g // NCH) * H + p * 16 + k, _pk_rows(g, db * 8, 8), :] = (
            pltpu.bitcast(t[k], u32))

  def pro_dot(g, wsrc, may_be_first, b, h):
    m, kc = g // NCH, g % NCH
    rows = pl.ds(RING0 + b * PRB, PRB)
    part = _dot(_bf(xnp[kc, pl.ds(b * (PRB // 2), PRB // 2), :]),
                _bf(wsrc[m * H + h, _pk_rows(g, 0, DCH // 2), :]))
    dst = qkvbuf[h].at[m]
    old = dst[rows, :]
    if may_be_first:
      old = jnp.where(kc == 0, np.float32(0), old)
    dst[rows, :] = old + part

  NB = XP // PRB

  def pro_half(g, wsrc, half, may_be_first):
    for b in range(half * NB // 2, (half + 1) * NB // 2):
      for h in range(H):
        pro_dot(g, wsrc, may_be_first, b, h)

  NG = 3 * NCH
  def stage_wait_if(g):
    pl.when(g < NG)(lambda: stage_wait(g))

  stage_wait(0)
  relayout(0, wqa)
  stage_start(NSLOT)
  pro_half(0, wqa, 0, True)
  stage_wait(1)
  stage_wait(2)

  def pro_body(i, _):
    g = 2 * i
    pro_half(g, wqa, 1, True)
    relayout(g + 1, wqb)
    pro_half(g + 1, wqb, 0, False)
    pro_half(g + 1, wqb, 1, False)
    relayout(g + 2, wqa)
    pro_half(g + 2, wqa, 0, True)
    stage_start(g + NSLOT + 1)
    stage_start(g + NSLOT + 2)

    @pl.when(i < 8)
    def _():
      for name, j in (("wo", i), ("w1", i), ("w2", i), ("w3", 2 * i), ("w3", 2 * i + 1)):
        strip(name, j).start()

    @pl.when(i == 8)
    def _():
      xb_cp.start()
      for j in range(16, 24):
        strip("w3", j).start()

    @pl.when(i == 9)
    def _():
      for j in range(24, 28):
        strip("w3", j).start()
      for j in range(4):
        strip("w4", j).start()

    @pl.when(i == 10)
    def _():
      for j in range(4, 8):
        strip("w4", j).start()

    stage_wait(g + 3)
    stage_wait_if(g + 4)
    return 0

  lax.fori_loop(0, NG // 2 - 1, pro_body, 0)
  pro_half(NG - 2, wqa, 1, False)
  relayout(NG - 1, wqb)
  pro_half(NG - 1, wqb, 0, False)
  pro_half(NG - 1, wqb, 1, False)

  row = lax.broadcasted_iota(jnp.int32, (L, L), 0)
  col = lax.broadcasted_iota(jnp.int32, (L, L), 1)
  mask = (row < M) | (col <= row)

  def st_xn(s):
    xs = xv[_rows(XP + s * RX, RX), :].astype(f32)
    xnbuf[s % 2] = _ln(xs)

  def wrow(s):
    return _rows(((s + (XP + RING0) // RX) % (RING // RX)) * RX, RX)

  def rrow(s):
    return _rows(((s + RING0 // seg) % (RING // seg)) * seg, seg)

  def st_lhs(s):
    return jnp.concatenate([membuf[...], xnbuf[s % 2]], axis=0).astype(bf16)

  def st_qkv(s, lhs, h, m):
    half = DCH // 2
    w = jnp.concatenate(
        [(wqa, wqb)[kc % 2][m * H + h, pl.ds((kc // 2) * half, half), :]
         for kc in range(NCH)], axis=0)
    r = _dot(lhs, _bf(w))
    qkvbuf[h][m, wrow(s), :] = r[M:]
    return r[:M]

  def ld(s, h, m, fresh):
    return jnp.concatenate([fresh, qkvbuf[h][m, rrow(s), :]], axis=0)

  def st_scores(q, k):
    return _dot_nt(q, k.astype(bf16))

  def st_softmax(sc):
    t = jnp.where(mask, sc * np.float32(scale * LOG2E), np.float32(-1e9 * LOG2E))
    e = jnp.exp2(t - jnp.max(t, axis=-1, keepdims=True))
    l = jnp.sum(e, axis=-1, keepdims=True)
    r = pl.reciprocal(l, approx=True)
    r = r * (2.0 - l * r)
    return e * r

  def st_pv(h, p, v):
    obuf[:, h * E:(h + 1) * E] = _dot(p, v.astype(bf16))

  def st_wo(s, j):
    r = _dot(obuf[...], _bf(wo[j]))
    membuf[:, j * 128:(j + 1) * 128] = r[:M]
    abuf[:, j * 128:(j + 1) * 128] = r[M:]

  def st_post(t):
    xs = xv[_rows(t * seg, seg), :].astype(f32)
    ha = xs + abuf[...]
    habuf[t % 4] = ha
    y = _ln(ha)
    ybuf[t % 4] = y
    zbuf[0] = _pk(_ln(y))

  def st_b1(t, j):
    g = _gelu(_dot(_bf(zbuf[0]), _bf(w1[j])))
    h1buf[_rows(PAD + t * seg, seg), j * 128:(j + 1) * 128] = g

  c4 = D // 4

  def st_shift(t):
    win = h1buf[_rows(t * seg, seg + 2 * PAD), :]
    g0 = win[PAD - 1:PAD - 1 + seg, 0 * c4:1 * c4]
    g1 = win[PAD + 1:PAD + 1 + seg, 1 * c4:2 * c4]
    g2 = win[PAD - 2:PAD - 2 + seg, 2 * c4:3 * c4]
    g3 = win[PAD + 2:PAD + 2 + seg, 3 * c4:4 * c4]
    zbuf[1] = _pk(jnp.concatenate([g0, g1, g2, g3], axis=1))

  def st_b2(t, j):
    cs = slice(j * 128, (j + 1) * 128)
    x1buf[:, cs] = ybuf[t % 4, :, cs] + _dot(_bf(zbuf[1]), _bf(w2[j]))

  def st_ln2(t):
    zbuf[2] = _pk(_ln(x1buf[...]))

  def st_b3(t, j):
    gbuf[:, j * 128:(j + 1) * 128] = _pk(_gelu(_dot(_bf(zbuf[2]), _bf(w3[j]))))

  def st_b4(t, j):
    cs = slice(j * 128, (j + 1) * 128)
    h2 = _dot(_bf(gbuf[...]), _bf(w4[j]))
    res = habuf[t % 4, :, cs] + (x1buf[:, cs] + h2)
    outv[_rows(t * seg, seg), cs] = res.astype(outv.dtype)

  def st_out(t):
    r = _rows(t * seg, seg)
    pltpu.make_async_copy(outv.at[r], out_hbm.at[r], sems.at[7]).start()

  def step(s, do_r, do_b1, do_b2, waits=()):
    waits = dict(waits)
    t1, t2 = s - 1, s - 2
    nf3 = F // 128
    ops = {}

    def wait(name):
      for cp in waits.get(name, ()):
        cp.wait()

    if do_r:
      fresh, probs = {}, {}
      lhs = st_lhs(s)
      heads = lambda g: range(g * HG, (g + 1) * HG)

      def op_q(g):
        for h in heads(g):
          fresh[h] = [st_qkv(s, lhs, h, m) for m in range(3)]

      def op_s(g):
        sc = [st_scores(ld(s, h, 0, fresh[h][0]), ld(s, h, 1, fresh[h][1]))
              for h in heads(g)]
        for h, v in zip(heads(g), sc):
          probs[h] = st_softmax(v)

      def op_p(g):
        vs = [ld(s, h, 2, fresh.pop(h)[2]) for h in heads(g)]
        for h, v in zip(heads(g), vs):
          st_pv(h, probs.pop(h), v)

      def op_xn():
        if isinstance(s, int):
          if s + 1 < nseg:
            st_xn(s + 1)
        else:
          st_xn(jnp.minimum(s + 1, nseg - 1))

      def op_wo(js):
        if js[0] == 0:
          wait("wo")
        for j in js:
          st_wo(s, j)

      for g in range(H // HG):
        ops[f"Q{g}"] = functools.partial(op_q, g)
        ops[f"S{g}"] = functools.partial(op_s, g)
        ops[f"P{g}"] = functools.partial(op_p, g)
      ops["XN"] = op_xn
      ops["WO"] = lambda: op_wo(range(8))

    if do_b1:
      def op_b1():
        wait("w1")
        for j in range(8):
          st_b1(t1, j)
      ops["POST"] = lambda: st_post(t1)
      ops["B1"] = op_b1

    if do_b2:
      def op_b2():
        wait("w2")
        st_shift(t2)
        for j in range(8):
          st_b2(t2, j)
        st_ln2(t2)

      def op_b3(js):
        if js[0] == 0:
          wait("w3")
        for j in js:
          st_b3(t2, j)

      def op_b4(js):
        if js[0] == 0:
          wait("w4")
        for j in js:
          st_b4(t2, j)
        if js[-1] == 7:
          st_out(t2)

      ops["B2"] = op_b2
      ops["B3a"] = lambda: op_b3(range(0, nf3 // 2))
      ops["B3b"] = lambda: op_b3(range(nf3 // 2, nf3))
      ops["B4a"] = lambda: op_b4(range(0, 3))
      ops["B4b"] = lambda: op_b4(range(3, 6))
      ops["B4c"] = lambda: op_b4(range(6, 8))

    for name in SCHEDULE.split():
      if name in ops:
        ops.pop(name)()
    assert not ops, ops

  xb_cp.wait()
  st_xn(0)
  step(0, True, False, False, waits={"wo": strips("wo")})
  step(1, True, True, False, waits={"w1": strips("w1")})
  step(2, True, True, True, waits={n: strips(n) for n in ("w2", "w3", "w4")})

  first = 3 + (nseg - 3) % UNROLL
  for s in range(3, first):
    step(s, True, True, True)

  def body(i, _):
    for u in range(UNROLL):
      step(first + i * UNROLL + u, True, True, True)
    return 0

  lax.fori_loop(0, (nseg - first) // UNROLL, body, 0)
  step(nseg, False, True, True)
  step(nseg + 1, False, False, True)
  pltpu.make_async_copy(outv, out_hbm, sems.at[7]).wait()


def _forward(A_x, A_mem0, A_Wq, A_Wk, A_Wv, A_Wo, seg, B_w1, B_w2, B_w3, B_w4):
  assert A_x.shape == (1, S, D) and A_mem0.shape == (1, M, D)
  assert A_Wq.shape == (D, H, E) and A_Wo.shape == (H, E, D) and B_w3.shape == (D, F)
  assert seg == 32 and XP + (S // seg) * RX == S
  x2 = A_x.reshape(S, D)
  mem0 = A_mem0.reshape(M, D)
  wq, wk, wv = A_Wq, A_Wk, A_Wv
  wo = A_Wo.reshape(H * E, D)
  any_spec = pl.BlockSpec(memory_space=pl.ANY)
  scratch = [
      pltpu.VMEM((S, D), bf16),
      pltpu.VMEM((3 * H, D // 4, E), u32),
      pltpu.VMEM((3 * H, D // 4, E), u32),
      pltpu.VMEM((D // 128, H * E // 2, 128), u32),
      pltpu.VMEM((D // 128, D // 2, 128), u32),
      pltpu.VMEM((D // 128, D // 2, 128), u32),
      pltpu.VMEM((F // 128, D // 2, 128), u32),
      pltpu.VMEM((D // 128, F // 2, 128), u32),
      pltpu.VMEM((NSLOT, DCH, H // 2, E), u32),
      pltpu.VMEM((NCH, XP // 2, 128), u32),
      [pltpu.VMEM((3, RING, E), f32) for _ in range(H)],
      pltpu.VMEM((M, D), f32),
      pltpu.VMEM((2, RX, D), f32),
      pltpu.VMEM((M + seg, H * E), f32),
      pltpu.VMEM((seg, D), f32),
      pltpu.VMEM((4, seg, D), f32),
      pltpu.VMEM((4, seg, D), f32),
      pltpu.VMEM((S + 2 * PAD, D), f32),
      pltpu.VMEM((seg, D), f32),
      pltpu.VMEM((3, seg // 2, D), u32),
      pltpu.VMEM((seg // 2, F), u32),
      pltpu.VMEM((S, D), A_x.dtype),
      pltpu.SemaphoreType.DMA((NSLOT,)),
      pltpu.SemaphoreType.DMA((8,)),
  ]
  out = pl.pallas_call(
      functools.partial(_kernel, seg),
      out_shape=jax.ShapeDtypeStruct((S, D), A_x.dtype),
      in_specs=[any_spec, pl.BlockSpec(memory_space=pltpu.VMEM)] + [any_spec] * 8,
      out_specs=any_spec,
      scratch_shapes=scratch,
      compiler_params=pltpu.CompilerParams(vmem_limit_bytes=126 * 2**20),
  )(x2, mem0, wq, wk, wv, wo, B_w1, B_w2, B_w3, B_w4)
  return out.reshape(1, S, D)


def pallas_sequential_preLN__memory_aug_recurrent_mem_tr__mixer_s_mlp__prompt_kernel(
    A_x, A_mem0, A_Wq, A_Wk, A_Wv, A_Wo, A_seg_len, B_x, B_w1, B_w2, B_w3, B_w4):
  del B_x
  return _forward(A_x, A_mem0, A_Wq, A_Wk, A_Wv, A_Wo, int(A_seg_len),
                  B_w1, B_w2, B_w3, B_w4)
```

```python
import functools

import jax
import jax.numpy as jnp
import numpy as np
from jax import lax
from jax.experimental import pallas as pl
from jax.experimental.pallas import tpu as pltpu

f32, bf16, u32 = jnp.float32, jnp.bfloat16, jnp.uint32

S, D, H, E, M, F = 2048, 1024, 32, 128, 8, 3584
LN_EPS = 1e-5
LOG2E = float(np.log2(np.e))
DCH = 128
NCH = D // DCH
NSLOT = 6
PAD = 8
XP = 512
PRB = 128
RX = 24
RING = 768
UNROLL = 1
HG = 4
SCHEDULE = """
    POST Q0 Q1 S0 B1 Q2 S1 P0 B2 Q3 S2 P1 B3a Q4 S3 P2 B3b Q5 S4 P3 Q6 S5 P4 B4a
    Q7 S6 P5 XN B4b S7 P6 B4c P7 WO
"""
RING0 = 64


def _dot(a, b):
  return lax.dot_general(a, b, (((1,), (0,)), ((), ())), preferred_element_type=f32)


def _dot_nt(a, b):
  return lax.dot_general(a, b, (((1,), (1,)), ((), ())), preferred_element_type=f32)


def _bf(w):
  return pltpu.bitcast(w, bf16)


def _pk(x):
  return pltpu.bitcast(x.astype(bf16), u32)


def _ln(x):
  m = jnp.mean(x, axis=-1, keepdims=True)
  d = x - m
  v = jnp.mean(d * d, axis=-1, keepdims=True)
  return d * lax.rsqrt(v + LN_EPS)


def _gelu(x):
  c = np.float32(np.sqrt(2.0 / np.pi))
  inner = x * (c + (np.float32(c * 0.044715)) * (x * x))
  return (0.5 * x) * (1.0 + jnp.tanh(inner))


def _rows(i, n):
  if isinstance(i, int):
    return pl.ds(i, n)
  return pl.ds(pl.multiple_of(i, 8), n)


def _kernel(seg, x_hbm, mem0_hbm, wq_hbm, wk_hbm, wv_hbm, wo_hbm, w1_hbm, w2_hbm,
            w3_hbm, w4_hbm, out_hbm,
            xv, mem0v, wqa, wqb, wo, w1, w2, w3, w4, stage, xnp, qkvbuf, membuf, xnbuf,
            obuf, abuf, ybuf, habuf, h1buf, x1buf, zbuf, gbuf, outv, st_sem, sems):
  nseg = S // seg
  L = M + seg
  scale = np.float32(E ** -0.5)

  xa_cp = pltpu.make_async_copy(x_hbm.at[0:XP], xv.at[0:XP], sems.at[0])
  xb_cp = pltpu.make_async_copy(x_hbm.at[XP:S], xv.at[XP:S], sems.at[6])
  qkv_hbm = (wq_hbm, wk_hbm, wv_hbm)

  def stage_cp(m, c, slot):
    src = qkv_hbm[m].at[pl.ds(c * DCH, DCH)]
    return pltpu.make_async_copy(src, stage.at[slot].bitcast(bf16), st_sem.at[slot])

  def stage_wait(g):
    stage_cp(0, 0, g % NSLOT).wait()

  def stage_start(g):
    for m in range(3):
      if isinstance(g, int):
        if m * NCH <= g < (m + 1) * NCH:
          stage_cp(m, g - m * NCH, g % NSLOT).start()
      else:
        @pl.when((g >= m * NCH) & (g < (m + 1) * NCH))
        def _(m=m):
          stage_cp(m, g - m * NCH, g % NSLOT).start()

  strip_src = {"wo": (wo_hbm, wo, 1), "w1": (w1_hbm, w1, 2), "w2": (w2_hbm, w2, 3),
               "w3": (w3_hbm, w3, 4), "w4": (w4_hbm, w4, 5)}

  def strip(name, j):
    w_hbm, dst, sem = strip_src[name]
    col = j * 128 if isinstance(j, int) else pl.multiple_of(j * 128, 128)
    return pltpu.make_async_copy(
        w_hbm.at[:, pl.ds(col, 128)], dst.at[j].bitcast(bf16), sems.at[sem])

  def strips(name):
    return [strip(name, j) for j in range(strip_src[name][1].shape[0])]

  mem0_cp = pltpu.make_async_copy(mem0_hbm, mem0v, sems.at[8])
  mem0_cp.start()
  xa_cp.start()
  stage_start(0)
  h1buf[0:PAD, :] = jnp.zeros((PAD, D), f32)
  h1buf[PAD + S:PAD + S + PAD, :] = jnp.zeros((PAD, D), f32)

  mem0_cp.wait()
  membuf[...] = mem0v[...].astype(f32)
  for g in range(1, NSLOT):
    stage_start(g)
  xa_cp.wait()
  LNB = 64
  for i in range(XP // LNB):
    r = pl.ds(i * LNB, LNB)
    xn = _pk(_ln(xv[r, :].astype(f32)))
    for kc in range(NCH):
      xnp[kc, pl.ds(i * (LNB // 2), LNB // 2), :] = xn[:, kc * 128:(kc + 1) * 128]

  def _pk_rows(g, off, n):
    return _rows(((g % NCH) // 2) * (DCH // 2) + off, n)

  NU = 2 * DCH // 16

  def relayout(g, wdst, units=range(NU)):
    for u in units:
      db, p = u // 2, u % 2
      v = _bf(stage[g % NSLOT, pl.ds(db * 16, 16), pl.ds(p * 8, 8), :])
      t = jnp.swapaxes(v, 0, 1)
      for k in range(16):
        wdst[(g // NCH) * H + p * 16 + k, _pk_rows(g, db * 8, 8), :] = (
            pltpu.bitcast(t[k], u32))

  def pro_dot(g, wsrc, may_be_first, b, h):
    m, kc = g // NCH, g % NCH
    rows = pl.ds(RING0 + b * PRB, PRB)
    part = _dot(_bf(xnp[kc, pl.ds(b * (PRB // 2), PRB // 2), :]),
                _bf(wsrc[m * H + h, _pk_rows(g, 0, DCH // 2), :]))
    dst = qkvbuf[h].at[m]
    old = dst[rows, :]
    if may_be_first:
      old = jnp.where(kc == 0, np.float32(0), old)
    dst[rows, :] = old + part

  NB = XP // PRB

  def pro_half(g, wsrc, half, may_be_first):
    for b in range(half * NB // 2, (half + 1) * NB // 2):
      for h in range(H):
        pro_dot(g, wsrc, may_be_first, b, h)

  NG = 3 * NCH
  def stage_wait_if(g):
    pl.when(g < NG)(lambda: stage_wait(g))

  stage_wait(0)
  relayout(0, wqa)
  stage_start(NSLOT)
  pro_half(0, wqa, 0, True)
  pro_half(0, wqa, 1, True)
  stage_wait(1)
  relayout(1, wqb)
  stage_start(NSLOT + 1)
  pro_half(1, wqb, 0, False)
  stage_wait(2)
  stage_wait(3)

  def pro_body(i, _):
    g = 2 * i + 1
    pro_half(g, wqb, 1, False)
    relayout(g + 1, wqa)
    pro_half(g + 1, wqa, 0, True)
    pro_half(g + 1, wqa, 1, True)
    relayout(g + 2, wqb)
    pro_half(g + 2, wqb, 0, False)
    stage_start(g + NSLOT + 1)
    stage_start(g + NSLOT + 2)

    @pl.when(i < 8)
    def _():
      for name, j in (("wo", i), ("w1", i), ("w2", i), ("w3", 2 * i), ("w3", 2 * i + 1)):
        strip(name, j).start()

    @pl.when(i == 8)
    def _():
      xb_cp.start()
      for j in range(16, 24):
        strip("w3", j).start()

    @pl.when(i == 9)
    def _():
      for j in range(24, 28):
        strip("w3", j).start()
      for j in range(4):
        strip("w4", j).start()

    @pl.when(i == 10)
    def _():
      for j in range(4, 8):
        strip("w4", j).start()

    stage_wait_if(g + 3)
    stage_wait_if(g + 4)
    return 0

  lax.fori_loop(0, NG // 2 - 1, pro_body, 0)
  pro_half(NG - 1, wqb, 1, False)

  row = lax.broadcasted_iota(jnp.int32, (L, L), 0)
  col = lax.broadcasted_iota(jnp.int32, (L, L), 1)
  mask = (row < M) | (col <= row)

  def st_xn(s):
    xs = xv[_rows(XP + s * RX, RX), :].astype(f32)
    xnbuf[s % 2] = _ln(xs)

  def wrow(s):
    return _rows(((s + (XP + RING0) // RX) % (RING // RX)) * RX, RX)

  def rrow(s):
    return _rows(((s + RING0 // seg) % (RING // seg)) * seg, seg)

  def st_lhs(s):
    return jnp.concatenate([membuf[...], xnbuf[s % 2]], axis=0).astype(bf16)

  def st_qkv(s, lhs, h, m):
    half = DCH // 2
    w = jnp.concatenate(
        [(wqa, wqb)[kc % 2][m * H + h, pl.ds((kc // 2) * half, half), :]
         for kc in range(NCH)], axis=0)
    r = _dot(lhs, _bf(w))
    qkvbuf[h][m, wrow(s), :] = r[M:]
    return r[:M]

  def ld(s, h, m, fresh):
    return jnp.concatenate([fresh, qkvbuf[h][m, rrow(s), :]], axis=0)

  def st_scores(q, k):
    return _dot_nt(q, k.astype(bf16))

  def st_softmax(sc):
    t = jnp.where(mask, sc * np.float32(scale * LOG2E), np.float32(-1e9 * LOG2E))
    e = jnp.exp2(t - jnp.max(t, axis=-1, keepdims=True))
    l = jnp.sum(e, axis=-1, keepdims=True)
    r = pl.reciprocal(l, approx=True)
    r = r * (2.0 - l * r)
    return e * r

  def st_pv(h, p, v):
    obuf[:, h * E:(h + 1) * E] = _dot(p, v.astype(bf16))

  def st_wo(s, j):
    r = _dot(obuf[...], _bf(wo[j]))
    membuf[:, j * 128:(j + 1) * 128] = r[:M]
    abuf[:, j * 128:(j + 1) * 128] = r[M:]

  def st_post(t):
    xs = xv[_rows(t * seg, seg), :].astype(f32)
    ha = xs + abuf[...]
    habuf[t % 4] = ha
    y = _ln(ha)
    ybuf[t % 4] = y
    zbuf[0] = _pk(_ln(y))

  def st_b1(t, j):
    g = _gelu(_dot(_bf(zbuf[0]), _bf(w1[j])))
    h1buf[_rows(PAD + t * seg, seg), j * 128:(j + 1) * 128] = g

  c4 = D // 4

  def st_shift(t):
    win = h1buf[_rows(t * seg, seg + 2 * PAD), :]
    g0 = win[PAD - 1:PAD - 1 + seg, 0 * c4:1 * c4]
    g1 = win[PAD + 1:PAD + 1 + seg, 1 * c4:2 * c4]
    g2 = win[PAD - 2:PAD - 2 + seg, 2 * c4:3 * c4]
    g3 = win[PAD + 2:PAD + 2 + seg, 3 * c4:4 * c4]
    zbuf[1] = _pk(jnp.concatenate([g0, g1, g2, g3], axis=1))

  def st_b2(t, j):
    cs = slice(j * 128, (j + 1) * 128)
    x1buf[:, cs] = ybuf[t % 4, :, cs] + _dot(_bf(zbuf[1]), _bf(w2[j]))

  def st_ln2(t):
    zbuf[2] = _pk(_ln(x1buf[...]))

  def st_b3(t, j):
    gbuf[:, j * 128:(j + 1) * 128] = _pk(_gelu(_dot(_bf(zbuf[2]), _bf(w3[j]))))

  def st_b4(t, j):
    cs = slice(j * 128, (j + 1) * 128)
    h2 = _dot(_bf(gbuf[...]), _bf(w4[j]))
    res = habuf[t % 4, :, cs] + (x1buf[:, cs] + h2)
    outv[_rows(t * seg, seg), cs] = res.astype(outv.dtype)

  def st_out(t):
    r = _rows(t * seg, seg)
    pltpu.make_async_copy(outv.at[r], out_hbm.at[r], sems.at[7]).start()

  def step(s, do_r, do_b1, do_b2, waits=()):
    waits = dict(waits)
    t1, t2 = s - 1, s - 2
    nf3 = F // 128
    ops = {}

    def wait(name):
      for cp in waits.get(name, ()):
        cp.wait()

    if do_r:
      fresh, probs = {}, {}
      lhs = st_lhs(s)
      heads = lambda g: range(g * HG, (g + 1) * HG)

      def op_q(g):
        for h in heads(g):
          fresh[h] = [st_qkv(s, lhs, h, m) for m in range(3)]

      def op_s(g):
        sc = [st_scores(ld(s, h, 0, fresh[h][0]), ld(s, h, 1, fresh[h][1]))
              for h in heads(g)]
        for h, v in zip(heads(g), sc):
          probs[h] = st_softmax(v)

      def op_p(g):
        vs = [ld(s, h, 2, fresh.pop(h)[2]) for h in heads(g)]
        for h, v in zip(heads(g), vs):
          st_pv(h, probs.pop(h), v)

      def op_xn():
        if isinstance(s, int):
          if s + 1 < nseg:
            st_xn(s + 1)
        else:
          st_xn(jnp.minimum(s + 1, nseg - 1))

      def op_wo(js):
        if js[0] == 0:
          wait("wo")
        for j in js:
          st_wo(s, j)

      for g in range(H // HG):
        ops[f"Q{g}"] = functools.partial(op_q, g)
        ops[f"S{g}"] = functools.partial(op_s, g)
        ops[f"P{g}"] = functools.partial(op_p, g)
      ops["XN"] = op_xn
      ops["WO"] = lambda: op_wo(range(8))

    if do_b1:
      def op_b1():
        wait("w1")
        for j in range(8):
          st_b1(t1, j)
      ops["POST"] = lambda: st_post(t1)
      ops["B1"] = op_b1

    if do_b2:
      def op_b2():
        wait("w2")
        st_shift(t2)
        for j in range(8):
          st_b2(t2, j)
        st_ln2(t2)

      def op_b3(js):
        if js[0] == 0:
          wait("w3")
        for j in js:
          st_b3(t2, j)

      def op_b4(js):
        if js[0] == 0:
          wait("w4")
        for j in js:
          st_b4(t2, j)
        if js[-1] == 7:
          st_out(t2)

      ops["B2"] = op_b2
      ops["B3a"] = lambda: op_b3(range(0, nf3 // 2))
      ops["B3b"] = lambda: op_b3(range(nf3 // 2, nf3))
      ops["B4a"] = lambda: op_b4(range(0, 3))
      ops["B4b"] = lambda: op_b4(range(3, 6))
      ops["B4c"] = lambda: op_b4(range(6, 8))

    for name in SCHEDULE.split():
      if name in ops:
        ops.pop(name)()
    assert not ops, ops

  xb_cp.wait()
  st_xn(0)
  step(0, True, False, False, waits={"wo": strips("wo")})
  step(1, True, True, False, waits={"w1": strips("w1")})
  step(2, True, True, True, waits={n: strips(n) for n in ("w2", "w3", "w4")})

  first = 3 + (nseg - 3) % UNROLL
  for s in range(3, first):
    step(s, True, True, True)

  def body(i, _):
    for u in range(UNROLL):
      step(first + i * UNROLL + u, True, True, True)
    return 0

  lax.fori_loop(0, (nseg - first) // UNROLL, body, 0)
  step(nseg, False, True, True)
  step(nseg + 1, False, False, True)
  pltpu.make_async_copy(outv, out_hbm, sems.at[7]).wait()


def _forward(A_x, A_mem0, A_Wq, A_Wk, A_Wv, A_Wo, seg, B_w1, B_w2, B_w3, B_w4):
  assert A_x.shape == (1, S, D) and A_mem0.shape == (1, M, D)
  assert A_Wq.shape == (D, H, E) and A_Wo.shape == (H, E, D) and B_w3.shape == (D, F)
  assert seg == 32 and XP + (S // seg) * RX == S
  x2 = A_x.reshape(S, D)
  mem0 = A_mem0.reshape(M, D)
  wq, wk, wv = A_Wq, A_Wk, A_Wv
  wo = A_Wo.reshape(H * E, D)
  any_spec = pl.BlockSpec(memory_space=pl.ANY)
  scratch = [
      pltpu.VMEM((S, D), bf16),
      pltpu.VMEM((M, D), bf16),
      pltpu.VMEM((3 * H, D // 4, E), u32),
      pltpu.VMEM((3 * H, D // 4, E), u32),
      pltpu.VMEM((D // 128, H * E // 2, 128), u32),
      pltpu.VMEM((D // 128, D // 2, 128), u32),
      pltpu.VMEM((D // 128, D // 2, 128), u32),
      pltpu.VMEM((F // 128, D // 2, 128), u32),
      pltpu.VMEM((D // 128, F // 2, 128), u32),
      pltpu.VMEM((NSLOT, DCH, H // 2, E), u32),
      pltpu.VMEM((NCH, XP // 2, 128), u32),
      [pltpu.VMEM((3, RING, E), f32) for _ in range(H)],
      pltpu.VMEM((M, D), f32),
      pltpu.VMEM((2, RX, D), f32),
      pltpu.VMEM((M + seg, H * E), f32),
      pltpu.VMEM((seg, D), f32),
      pltpu.VMEM((4, seg, D), f32),
      pltpu.VMEM((4, seg, D), f32),
      pltpu.VMEM((S + 2 * PAD, D), f32),
      pltpu.VMEM((seg, D), f32),
      pltpu.VMEM((3, seg // 2, D), u32),
      pltpu.VMEM((seg // 2, F), u32),
      pltpu.VMEM((S, D), A_x.dtype),
      pltpu.SemaphoreType.DMA((NSLOT,)),
      pltpu.SemaphoreType.DMA((9,)),
  ]
  out = pl.pallas_call(
      functools.partial(_kernel, seg),
      out_shape=jax.ShapeDtypeStruct((S, D), A_x.dtype),
      in_specs=[any_spec] * 10,
      out_specs=any_spec,
      scratch_shapes=scratch,
      compiler_params=pltpu.CompilerParams(vmem_limit_bytes=126 * 2**20),
  )(x2, mem0, wq, wk, wv, wo, B_w1, B_w2, B_w3, B_w4)
  return out.reshape(1, S, D)


def pallas_sequential_preLN__memory_aug_recurrent_mem_tr__mixer_s_mlp__prompt_kernel(
    A_x, A_mem0, A_Wq, A_Wk, A_Wv, A_Wo, A_seg_len, B_x, B_w1, B_w2, B_w3, B_w4):
  del B_x
  return _forward(A_x, A_mem0, A_Wq, A_Wk, A_Wv, A_Wo, int(A_seg_len),
                  B_w1, B_w2, B_w3, B_w4)
```

```python
import functools

import jax
import jax.numpy as jnp
import numpy as np
from jax import lax
from jax.experimental import pallas as pl
from jax.experimental.pallas import tpu as pltpu

f32, bf16, u32 = jnp.float32, jnp.bfloat16, jnp.uint32

S, D, H, E, M, F = 2048, 1024, 32, 128, 8, 3584
LN_EPS = 1e-5
LOG2E = float(np.log2(np.e))
DCH = 128
NCH = D // DCH
NSLOT = 6
PAD = 8
XP = 512
PRB = 128
RX = 24
RING = 768
HG = 4
SCHEDULE = """
    POST Q0 Q1 S0 B1 Q2 S1 P0 B2 Q3 S2 P1 B3a Q4 S3 P2 B3b Q5 S4 P3 Q6 S5 P4 B4a
    Q7 S6 P5 XN B4b S7 P6 B4c P7 WO
"""
RING0 = 64


def _dot(a, b):
  return lax.dot_general(a, b, (((1,), (0,)), ((), ())), preferred_element_type=f32)


def _dot_nt(a, b):
  return lax.dot_general(a, b, (((1,), (1,)), ((), ())), preferred_element_type=f32)


def _bf(w):
  return pltpu.bitcast(w, bf16)


def _pk(x):
  return pltpu.bitcast(x.astype(bf16), u32)


def _ln(x):
  m = jnp.mean(x, axis=-1, keepdims=True)
  d = x - m
  v = jnp.mean(d * d, axis=-1, keepdims=True)
  return d * lax.rsqrt(v + LN_EPS)


def _gelu(x):
  c = np.float32(np.sqrt(2.0 / np.pi))
  inner = x * (c + (np.float32(c * 0.044715)) * (x * x))
  return (0.5 * x) * (1.0 + jnp.tanh(inner))


def _rows(i, n):
  if isinstance(i, int):
    return pl.ds(i, n)
  return pl.ds(pl.multiple_of(i, 8), n)


def _kernel(seg, x_hbm, mem0_hbm, wq_hbm, wk_hbm, wv_hbm, wo_hbm, w1_hbm, w2_hbm,
            w3_hbm, w4_hbm, out_hbm,
            xv, mem0v, wqa, wqb, wo, w1, w2, w3, w4, stage, xnp, qkvbuf, membuf, xnbuf,
            obuf, abuf, ybuf, habuf, h1buf, x1buf, zbuf, gbuf, outv, st_sem, sems):
  nseg = S // seg
  L = M + seg
  scale = np.float32(E ** -0.5)

  xa_cp = [pltpu.make_async_copy(x_hbm.at[r], xv.at[r], sems.at[k])
           for r, k in ((pl.ds(0, XP // 2), 0), (pl.ds(XP // 2, XP // 2), 9))]
  xb_cp = pltpu.make_async_copy(x_hbm.at[XP:S], xv.at[XP:S], sems.at[6])
  qkv_hbm = (wq_hbm, wk_hbm, wv_hbm)

  def stage_cp(m, c, slot):
    src = qkv_hbm[m].at[pl.ds(c * DCH, DCH)]
    return pltpu.make_async_copy(src, stage.at[slot].bitcast(bf16), st_sem.at[slot])

  def stage_wait(g):
    stage_cp(0, 0, g % NSLOT).wait()

  def stage_start(g):
    for m in range(3):
      if isinstance(g, int):
        if m * NCH <= g < (m + 1) * NCH:
          stage_cp(m, g - m * NCH, g % NSLOT).start()
      else:
        @pl.when((g >= m * NCH) & (g < (m + 1) * NCH))
        def _(m=m):
          stage_cp(m, g - m * NCH, g % NSLOT).start()

  strip_src = {"wo": (wo_hbm, wo, 1), "w1": (w1_hbm, w1, 2), "w2": (w2_hbm, w2, 3),
               "w3": (w3_hbm, w3, 4), "w4": (w4_hbm, w4, 5)}

  def strip(name, j):
    w_hbm, dst, sem = strip_src[name]
    col = j * 128 if isinstance(j, int) else pl.multiple_of(j * 128, 128)
    return pltpu.make_async_copy(
        w_hbm.at[:, pl.ds(col, 128)], dst.at[j].bitcast(bf16), sems.at[sem])

  def strips(name):
    return [strip(name, j) for j in range(strip_src[name][1].shape[0])]

  mem0_cp = pltpu.make_async_copy(mem0_hbm, mem0v, sems.at[8])
  mem0_cp.start()
  stage_start(0)
  h1buf[0:PAD, :] = jnp.zeros((PAD, D), f32)
  h1buf[PAD + S:PAD + S + PAD, :] = jnp.zeros((PAD, D), f32)

  mem0_cp.wait()
  membuf[...] = mem0v[...].astype(f32)
  for cp in xa_cp:
    cp.start()
  LNB = 64

  def ln_pro(half):
    xa_cp[half].wait()
    for i in range(half * XP // (2 * LNB), (half + 1) * XP // (2 * LNB)):
      xn = _pk(_ln(xv[pl.ds(i * LNB, LNB), :].astype(f32)))
      for kc in range(NCH):
        xnp[kc, pl.ds(i * (LNB // 2), LNB // 2), :] = xn[:, kc * 128:(kc + 1) * 128]

  def _pk_rows(g, off, n):
    return _rows(((g % NCH) // 2) * (DCH // 2) + off, n)

  NU = 2 * DCH // 16

  def relayout(g, wdst, units=range(NU)):
    for u in units:
      db, p = u // 2, u % 2
      v = _bf(stage[g % NSLOT, pl.ds(db * 16, 16), pl.ds(p * 8, 8), :])
      t = jnp.swapaxes(v, 0, 1)
      for k in range(16):
        wdst[(g // NCH) * H + p * 16 + k, _pk_rows(g, db * 8, 8), :] = (
            pltpu.bitcast(t[k], u32))

  def pro_dot(g, wsrc, may_be_first, b, h):
    m, kc = g // NCH, g % NCH
    rows = pl.ds(RING0 + b * PRB, PRB)
    part = _dot(_bf(xnp[kc, pl.ds(b * (PRB // 2), PRB // 2), :]),
                _bf(wsrc[m * H + h, _pk_rows(g, 0, DCH // 2), :]))
    dst = qkvbuf[h].at[m]
    old = dst[rows, :]
    if may_be_first:
      old = jnp.where(kc == 0, np.float32(0), old)
    dst[rows, :] = old + part

  NB = XP // PRB

  def pro_half(g, wsrc, half, may_be_first):
    for b in range(half * NB // 2, (half + 1) * NB // 2):
      for h in range(H):
        pro_dot(g, wsrc, may_be_first, b, h)

  NG = 3 * NCH
  def stage_wait_if(g):
    pl.when(g < NG)(lambda: stage_wait(g))

  stage_wait(0)
  for g in range(1, NSLOT):
    stage_start(g)
  relayout(0, wqa)
  stage_start(NSLOT)
  ln_pro(0)
  ln_pro(1)
  pro_half(0, wqa, 0, True)
  pro_half(0, wqa, 1, True)
  stage_wait(1)
  relayout(1, wqb)
  stage_start(NSLOT + 1)
  pro_half(1, wqb, 0, False)
  stage_wait(2)
  stage_wait(3)

  def pro_body(i, _):
    g = 2 * i + 1
    pro_half(g, wqb, 1, False)
    relayout(g + 1, wqa)
    pro_half(g + 1, wqa, 0, True)
    pro_half(g + 1, wqa, 1, True)
    relayout(g + 2, wqb)
    pro_half(g + 2, wqb, 0, False)
    stage_start(g + NSLOT + 1)
    stage_start(g + NSLOT + 2)

    @pl.when(i < 8)
    def _():
      for name, j in (("wo", i), ("w1", i), ("w2", i), ("w3", 2 * i), ("w3", 2 * i + 1)):
        strip(name, j).start()

    @pl.when(i == 8)
    def _():
      xb_cp.start()
      for j in range(16, 24):
        strip("w3", j).start()

    @pl.when(i == 9)
    def _():
      for j in range(24, 28):
        strip("w3", j).start()
      for j in range(4):
        strip("w4", j).start()

    @pl.when(i == 10)
    def _():
      for j in range(4, 8):
        strip("w4", j).start()

    stage_wait_if(g + 3)
    stage_wait_if(g + 4)
    return 0

  lax.fori_loop(0, NG // 2 - 1, pro_body, 0)
  pro_half(NG - 1, wqb, 1, False)

  row = lax.broadcasted_iota(jnp.int32, (L, L), 0)
  col = lax.broadcasted_iota(jnp.int32, (L, L), 1)
  mask = (row < M) | (col <= row)

  def st_xn(s):
    xs = xv[_rows(XP + s * RX, RX), :].astype(f32)
    xnbuf[s % 2] = _ln(xs)

  def wrow(s):
    return _rows(((s + (XP + RING0) // RX) % (RING // RX)) * RX, RX)

  def rrow(s):
    return _rows(((s + RING0 // seg) % (RING // seg)) * seg, seg)

  def st_lhs(s):
    return jnp.concatenate([membuf[...], xnbuf[s % 2]], axis=0).astype(bf16)

  def st_qkv(s, lhs, h, m):
    half = DCH // 2
    w = jnp.concatenate(
        [(wqa, wqb)[kc % 2][m * H + h, pl.ds((kc // 2) * half, half), :]
         for kc in range(NCH)], axis=0)
    r = _dot(lhs, _bf(w))
    qkvbuf[h][m, wrow(s), :] = r[M:]
    return r[:M]

  def ld(s, h, m, fresh):
    return jnp.concatenate([fresh, qkvbuf[h][m, rrow(s), :]], axis=0)

  def st_scores(q, k):
    return _dot_nt(q, k.astype(bf16))

  def st_softmax(sc):
    t = jnp.where(mask, sc * np.float32(scale * LOG2E), np.float32(-1e9 * LOG2E))
    e = jnp.exp2(t - jnp.max(t, axis=-1, keepdims=True))
    l = jnp.sum(e, axis=-1, keepdims=True)
    r = pl.reciprocal(l, approx=True)
    r = r * (2.0 - l * r)
    return e * r

  def st_pv(h, p, v):
    obuf[:, h * E:(h + 1) * E] = _dot(p, v.astype(bf16))

  def st_wo(s, j):
    r = _dot(obuf[...], _bf(wo[j]))
    membuf[:, j * 128:(j + 1) * 128] = r[:M]
    abuf[:, j * 128:(j + 1) * 128] = r[M:]

  def st_post(t):
    xs = xv[_rows(t * seg, seg), :].astype(f32)
    ha = xs + abuf[...]
    habuf[t % 4] = ha
    y = _ln(ha)
    ybuf[t % 4] = y
    zbuf[0] = _pk(_ln(y))

  def st_b1(t, j):
    g = _gelu(_dot(_bf(zbuf[0]), _bf(w1[j])))
    h1buf[_rows(PAD + t * seg, seg), j * 128:(j + 1) * 128] = g

  c4 = D // 4

  def st_shift(t):
    win = h1buf[_rows(t * seg, seg + 2 * PAD), :]
    g0 = win[PAD - 1:PAD - 1 + seg, 0 * c4:1 * c4]
    g1 = win[PAD + 1:PAD + 1 + seg, 1 * c4:2 * c4]
    g2 = win[PAD - 2:PAD - 2 + seg, 2 * c4:3 * c4]
    g3 = win[PAD + 2:PAD + 2 + seg, 3 * c4:4 * c4]
    zbuf[1] = _pk(jnp.concatenate([g0, g1, g2, g3], axis=1))

  def st_b2(t, j):
    cs = slice(j * 128, (j + 1) * 128)
    x1buf[:, cs] = ybuf[t % 4, :, cs] + _dot(_bf(zbuf[1]), _bf(w2[j]))

  def st_ln2(t):
    zbuf[2] = _pk(_ln(x1buf[...]))

  def st_b3(t, j):
    gbuf[:, j * 128:(j + 1) * 128] = _pk(_gelu(_dot(_bf(zbuf[2]), _bf(w3[j]))))

  def st_b4(t, j):
    cs = slice(j * 128, (j + 1) * 128)
    h2 = _dot(_bf(gbuf[...]), _bf(w4[j]))
    res = habuf[t % 4, :, cs] + (x1buf[:, cs] + h2)
    outv[_rows(t * seg, seg), cs] = res.astype(outv.dtype)

  def st_out(t):
    r = _rows(t * seg, seg)
    pltpu.make_async_copy(outv.at[r], out_hbm.at[r], sems.at[7]).start()

  def step(s, do_r, do_b1, do_b2):
    t1, t2 = s - 1, s - 2
    nf3 = F // 128
    ops = {}

    if do_r:
      fresh, probs = {}, {}
      lhs = st_lhs(s)
      heads = lambda g: range(g * HG, (g + 1) * HG)

      def op_q(g):
        for h in heads(g):
          fresh[h] = [st_qkv(s, lhs, h, m) for m in range(3)]

      def op_s(g):
        sc = [st_scores(ld(s, h, 0, fresh[h][0]), ld(s, h, 1, fresh[h][1]))
              for h in heads(g)]
        for h, v in zip(heads(g), sc):
          probs[h] = st_softmax(v)

      def op_p(g):
        vs = [ld(s, h, 2, fresh.pop(h)[2]) for h in heads(g)]
        for h, v in zip(heads(g), vs):
          st_pv(h, probs.pop(h), v)

      def op_xn():
        if isinstance(s, int):
          if s + 1 < nseg:
            st_xn(s + 1)
        else:
          st_xn(jnp.minimum(s + 1, nseg - 1))

      def op_wo(js):
        for j in js:
          st_wo(s, j)

      for g in range(H // HG):
        ops[f"Q{g}"] = functools.partial(op_q, g)
        ops[f"S{g}"] = functools.partial(op_s, g)
        ops[f"P{g}"] = functools.partial(op_p, g)
      ops["XN"] = op_xn
      ops["WO"] = lambda: op_wo(range(8))

    if do_b1:
      def op_b1():
        for j in range(8):
          st_b1(t1, j)
      ops["POST"] = lambda: st_post(t1)
      ops["B1"] = op_b1

    if do_b2:
      def op_b2():
        st_shift(t2)
        for j in range(8):
          st_b2(t2, j)
        st_ln2(t2)

      def op_b3(js):
        for j in js:
          st_b3(t2, j)

      def op_b4(js):
        for j in js:
          st_b4(t2, j)
        if js[-1] == 7:
          st_out(t2)

      ops["B2"] = op_b2
      ops["B3a"] = lambda: op_b3(range(0, nf3 // 2))
      ops["B3b"] = lambda: op_b3(range(nf3 // 2, nf3))
      ops["B4a"] = lambda: op_b4(range(0, 3))
      ops["B4b"] = lambda: op_b4(range(3, 6))
      ops["B4c"] = lambda: op_b4(range(6, 8))

    for name in SCHEDULE.split():
      if name in ops:
        ops.pop(name)()
    assert not ops, ops

  xb_cp.wait()
  for cp in strips("wo") + strips("w1"):
    cp.wait()
  st_xn(0)
  step(0, True, False, False)
  step(1, True, True, False)
  for cp in strips("w2") + strips("w3") + strips("w4"):
    cp.wait()

  def body(s, _):
    step(s, True, True, True)
    return 0

  lax.fori_loop(2, nseg, body, 0)
  step(nseg, False, True, True)
  step(nseg + 1, False, False, True)
  pltpu.make_async_copy(outv, out_hbm, sems.at[7]).wait()


def _forward(A_x, A_mem0, A_Wq, A_Wk, A_Wv, A_Wo, seg, B_w1, B_w2, B_w3, B_w4):
  assert A_x.shape == (1, S, D) and A_mem0.shape == (1, M, D)
  assert A_Wq.shape == (D, H, E) and A_Wo.shape == (H, E, D) and B_w3.shape == (D, F)
  assert seg == 32 and XP + (S // seg) * RX == S
  x2 = A_x.reshape(S, D)
  mem0 = A_mem0.reshape(M, D)
  wq, wk, wv = A_Wq, A_Wk, A_Wv
  wo = A_Wo.reshape(H * E, D)
  any_spec = pl.BlockSpec(memory_space=pl.ANY)
  scratch = [
      pltpu.VMEM((S, D), bf16),
      pltpu.VMEM((M, D), bf16),
      pltpu.VMEM((3 * H, D // 4, E), u32),
      pltpu.VMEM((3 * H, D // 4, E), u32),
      pltpu.VMEM((D // 128, H * E // 2, 128), u32),
      pltpu.VMEM((D // 128, D // 2, 128), u32),
      pltpu.VMEM((D // 128, D // 2, 128), u32),
      pltpu.VMEM((F // 128, D // 2, 128), u32),
      pltpu.VMEM((D // 128, F // 2, 128), u32),
      pltpu.VMEM((NSLOT, DCH, H // 2, E), u32),
      pltpu.VMEM((NCH, XP // 2, 128), u32),
      [pltpu.VMEM((3, RING, E), f32) for _ in range(H)],
      pltpu.VMEM((M, D), f32),
      pltpu.VMEM((2, RX, D), f32),
      pltpu.VMEM((M + seg, H * E), f32),
      pltpu.VMEM((seg, D), f32),
      pltpu.VMEM((4, seg, D), f32),
      pltpu.VMEM((4, seg, D), f32),
      pltpu.VMEM((S + 2 * PAD, D), f32),
      pltpu.VMEM((seg, D), f32),
      pltpu.VMEM((3, seg // 2, D), u32),
      pltpu.VMEM((seg // 2, F), u32),
      pltpu.VMEM((S, D), A_x.dtype),
      pltpu.SemaphoreType.DMA((NSLOT,)),
      pltpu.SemaphoreType.DMA((10,)),
  ]
  out = pl.pallas_call(
      functools.partial(_kernel, seg),
      out_shape=jax.ShapeDtypeStruct((S, D), A_x.dtype),
      in_specs=[any_spec] * 10,
      out_specs=any_spec,
      scratch_shapes=scratch,
      compiler_params=pltpu.CompilerParams(vmem_limit_bytes=126 * 2**20),
  )(x2, mem0, wq, wk, wv, wo, B_w1, B_w2, B_w3, B_w4)
  return out.reshape(1, S, D)


def pallas_sequential_preLN__memory_aug_recurrent_mem_tr__mixer_s_mlp__prompt_kernel(
    A_x, A_mem0, A_Wq, A_Wk, A_Wv, A_Wo, A_seg_len, B_x, B_w1, B_w2, B_w3, B_w4):
  del B_x
  return _forward(A_x, A_mem0, A_Wq, A_Wk, A_Wv, A_Wo, int(A_seg_len),
                  B_w1, B_w2, B_w3, B_w4)
```

```python
import functools

import jax
import jax.numpy as jnp
import numpy as np
from jax import lax
from jax.experimental import pallas as pl
from jax.experimental.pallas import tpu as pltpu

f32, bf16, u32 = jnp.float32, jnp.bfloat16, jnp.uint32

S, D, H, E, M, F = 2048, 1024, 32, 128, 8, 3584
LN_EPS = 1e-5
LOG2E = float(np.log2(np.e))
DCH = 128
NCH = D // DCH
NSLOT = 6
PAD = 8
XP = 512
PRB = 128
RX = 24
RING = 768
SCHEDULE = """
    POST Q:0-8 B1:0-8 Q:8-16 SHIFT B2:0-8 LN2 Q:16-24 B3:0-28 Q:24-32 XN
    B4:0-2 S:0-32 B4:2-5 P:0-32 B4:5-8 OUT WO:0-8
"""
RING0 = 64


def _dot(a, b):
  return lax.dot_general(a, b, (((1,), (0,)), ((), ())), preferred_element_type=f32)


def _dot_nt(a, b):
  return lax.dot_general(a, b, (((1,), (1,)), ((), ())), preferred_element_type=f32)


def _bf(w):
  return pltpu.bitcast(w, bf16)


def _pk(x):
  return pltpu.bitcast(x.astype(bf16), u32)


def _ln(x):
  m = jnp.mean(x, axis=-1, keepdims=True)
  d = x - m
  v = jnp.mean(d * d, axis=-1, keepdims=True)
  return d * lax.rsqrt(v + LN_EPS)


def _gelu(x):
  c = np.float32(np.sqrt(2.0 / np.pi))
  inner = x * (c + (np.float32(c * 0.044715)) * (x * x))
  return (0.5 * x) * (1.0 + jnp.tanh(inner))


def _rows(i, n):
  if isinstance(i, int):
    return pl.ds(i, n)
  return pl.ds(pl.multiple_of(i, 8), n)


def _kernel(seg, x_hbm, mem0_hbm, wq_hbm, wk_hbm, wv_hbm, wo_hbm, w1_hbm, w2_hbm,
            w3_hbm, w4_hbm, out_hbm,
            xv, mem0v, wqa, wqb, wo, w1, w2, w3, w4, stage, xnp, qkvbuf, membuf, xnbuf,
            obuf, abuf, ybuf, habuf, h1buf, x1buf, zbuf, gbuf, outv, st_sem, sems):
  nseg = S // seg
  L = M + seg
  scale = np.float32(E ** -0.5)

  xa_cp = [pltpu.make_async_copy(x_hbm.at[r], xv.at[r], sems.at[k])
           for r, k in ((pl.ds(0, XP // 2), 0), (pl.ds(XP // 2, XP // 2), 9))]
  xb_cp = pltpu.make_async_copy(x_hbm.at[XP:S], xv.at[XP:S], sems.at[6])
  qkv_hbm = (wq_hbm, wk_hbm, wv_hbm)

  def stage_cp(m, c, slot):
    src = qkv_hbm[m].at[pl.ds(c * DCH, DCH)]
    return pltpu.make_async_copy(src, stage.at[slot].bitcast(bf16), st_sem.at[slot])

  def stage_wait(g):
    stage_cp(0, 0, g % NSLOT).wait()

  def stage_start(g):
    for m in range(3):
      if isinstance(g, int):
        if m * NCH <= g < (m + 1) * NCH:
          stage_cp(m, g - m * NCH, g % NSLOT).start()
      else:
        @pl.when((g >= m * NCH) & (g < (m + 1) * NCH))
        def _(m=m):
          stage_cp(m, g - m * NCH, g % NSLOT).start()

  strip_src = {"wo": (wo_hbm, wo, 1), "w1": (w1_hbm, w1, 2), "w2": (w2_hbm, w2, 3),
               "w3": (w3_hbm, w3, 4), "w4": (w4_hbm, w4, 5)}

  def strip(name, j):
    w_hbm, dst, sem = strip_src[name]
    col = j * 128 if isinstance(j, int) else pl.multiple_of(j * 128, 128)
    return pltpu.make_async_copy(
        w_hbm.at[:, pl.ds(col, 128)], dst.at[j].bitcast(bf16), sems.at[sem])

  def strips(name):
    return [strip(name, j) for j in range(strip_src[name][1].shape[0])]

  mem0_cp = pltpu.make_async_copy(mem0_hbm, mem0v, sems.at[8])
  mem0_cp.start()
  stage_start(0)
  h1buf[0:PAD, :] = jnp.zeros((PAD, D), f32)
  h1buf[PAD + S:PAD + S + PAD, :] = jnp.zeros((PAD, D), f32)

  mem0_cp.wait()
  membuf[...] = mem0v[...].astype(f32)
  for cp in xa_cp:
    cp.start()
  LNB = 64

  def ln_pro(half):
    xa_cp[half].wait()
    for i in range(half * XP // (2 * LNB), (half + 1) * XP // (2 * LNB)):
      xn = _pk(_ln(xv[pl.ds(i * LNB, LNB), :].astype(f32)))
      for kc in range(NCH):
        xnp[kc, pl.ds(i * (LNB // 2), LNB // 2), :] = xn[:, kc * 128:(kc + 1) * 128]

  def _pk_rows(g, off, n):
    return _rows(((g % NCH) // 2) * (DCH // 2) + off, n)

  NU = 2 * DCH // 16

  def relayout(g, wdst, units=range(NU)):
    for u in units:
      db, p = u // 2, u % 2
      v = _bf(stage[g % NSLOT, pl.ds(db * 16, 16), pl.ds(p * 8, 8), :])
      t = jnp.swapaxes(v, 0, 1)
      for k in range(16):
        wdst[(g // NCH) * H + p * 16 + k, _pk_rows(g, db * 8, 8), :] = (
            pltpu.bitcast(t[k], u32))

  def pro_dot(g, wsrc, may_be_first, b, h):
    m, kc = g // NCH, g % NCH
    rows = pl.ds(RING0 + b * PRB, PRB)
    part = _dot(_bf(xnp[kc, pl.ds(b * (PRB // 2), PRB // 2), :]),
                _bf(wsrc[m * H + h, _pk_rows(g, 0, DCH // 2), :]))
    dst = qkvbuf[h].at[m]
    old = dst[rows, :]
    if may_be_first:
      old = jnp.where(kc == 0, np.float32(0), old)
    dst[rows, :] = old + part

  NB = XP // PRB

  def pro_half(g, wsrc, half, may_be_first):
    for b in range(half * NB // 2, (half + 1) * NB // 2):
      for h in range(H):
        pro_dot(g, wsrc, may_be_first, b, h)

  NG = 3 * NCH
  def stage_wait_if(g):
    pl.when(g < NG)(lambda: stage_wait(g))

  stage_wait(0)
  for g in range(1, NSLOT):
    stage_start(g)
  relayout(0, wqa)
  stage_start(NSLOT)
  ln_pro(0)
  ln_pro(1)
  pro_half(0, wqa, 0, True)
  pro_half(0, wqa, 1, True)
  stage_wait(1)
  relayout(1, wqb)
  stage_start(NSLOT + 1)
  pro_half(1, wqb, 0, False)
  stage_wait(2)
  stage_wait(3)

  def pro_body(i, _):
    g = 2 * i + 1
    pro_half(g, wqb, 1, False)
    relayout(g + 1, wqa)
    pro_half(g + 1, wqa, 0, True)
    pro_half(g + 1, wqa, 1, True)
    relayout(g + 2, wqb)
    pro_half(g + 2, wqb, 0, False)
    stage_start(g + NSLOT + 1)
    stage_start(g + NSLOT + 2)

    @pl.when(i < 8)
    def _():
      for name, j in (("wo", i), ("w1", i), ("w2", i), ("w3", 2 * i), ("w3", 2 * i + 1)):
        strip(name, j).start()

    @pl.when(i == 8)
    def _():
      xb_cp.start()
      for j in range(16, 24):
        strip("w3", j).start()

    @pl.when(i == 9)
    def _():
      for j in range(24, 28):
        strip("w3", j).start()
      for j in range(4):
        strip("w4", j).start()

    @pl.when(i == 10)
    def _():
      for j in range(4, 8):
        strip("w4", j).start()

    stage_wait_if(g + 3)
    stage_wait_if(g + 4)
    return 0

  lax.fori_loop(0, NG // 2 - 1, pro_body, 0)
  pro_half(NG - 1, wqb, 1, False)

  row = lax.broadcasted_iota(jnp.int32, (L, L), 0)
  col = lax.broadcasted_iota(jnp.int32, (L, L), 1)
  mask = (row < M) | (col <= row)

  def st_xn(s):
    xs = xv[_rows(XP + s * RX, RX), :].astype(f32)
    xnbuf[s % 2] = _ln(xs)

  def wrow(s):
    return _rows(((s + (XP + RING0) // RX) % (RING // RX)) * RX, RX)

  def rrow(s):
    return _rows(((s + RING0 // seg) % (RING // seg)) * seg, seg)

  def st_lhs(s):
    return jnp.concatenate([membuf[...], xnbuf[s % 2]], axis=0).astype(bf16)

  def st_qkv(s, lhs, h, m):
    half = DCH // 2
    w = jnp.concatenate(
        [(wqa, wqb)[kc % 2][m * H + h, pl.ds((kc // 2) * half, half), :]
         for kc in range(NCH)], axis=0)
    r = _dot(lhs, _bf(w))
    qkvbuf[h][m, wrow(s), :] = r[M:]
    return r[:M]

  def ld(s, h, m, fresh):
    return jnp.concatenate([fresh, qkvbuf[h][m, rrow(s), :]], axis=0)

  def st_scores(q, k):
    return _dot_nt(q, k.astype(bf16))

  def st_softmax(sc):
    t = jnp.where(mask, sc * np.float32(scale * LOG2E), np.float32(-1e9 * LOG2E))
    e = jnp.exp2(t - jnp.max(t, axis=-1, keepdims=True))
    l = jnp.sum(e, axis=-1, keepdims=True)
    r = pl.reciprocal(l, approx=True)
    r = r * (2.0 - l * r)
    return e * r

  def st_pv(h, p, v):
    obuf[:, h * E:(h + 1) * E] = _dot(p, v.astype(bf16))

  def st_wo(s, j):
    r = _dot(obuf[...], _bf(wo[j]))
    membuf[:, j * 128:(j + 1) * 128] = r[:M]
    abuf[:, j * 128:(j + 1) * 128] = r[M:]

  def st_post(t):
    xs = xv[_rows(t * seg, seg), :].astype(f32)
    ha = xs + abuf[...]
    habuf[t % 4] = ha
    y = _ln(ha)
    ybuf[t % 4] = y
    zbuf[0] = _pk(_ln(y))

  def st_b1(t, j):
    g = _gelu(_dot(_bf(zbuf[0]), _bf(w1[j])))
    h1buf[_rows(PAD + t * seg, seg), j * 128:(j + 1) * 128] = g

  c4 = D // 4

  def st_shift(t):
    win = h1buf[_rows(t * seg, seg + 2 * PAD), :]
    g0 = win[PAD - 1:PAD - 1 + seg, 0 * c4:1 * c4]
    g1 = win[PAD + 1:PAD + 1 + seg, 1 * c4:2 * c4]
    g2 = win[PAD - 2:PAD - 2 + seg, 2 * c4:3 * c4]
    g3 = win[PAD + 2:PAD + 2 + seg, 3 * c4:4 * c4]
    zbuf[1] = _pk(jnp.concatenate([g0, g1, g2, g3], axis=1))

  def st_b2(t, j):
    cs = slice(j * 128, (j + 1) * 128)
    x1buf[:, cs] = ybuf[t % 4, :, cs] + _dot(_bf(zbuf[1]), _bf(w2[j]))

  def st_ln2(t):
    zbuf[2] = _pk(_ln(x1buf[...]))

  def st_b3(t, j):
    gbuf[:, j * 128:(j + 1) * 128] = _pk(_gelu(_dot(_bf(zbuf[2]), _bf(w3[j]))))

  def st_b4(t, j):
    cs = slice(j * 128, (j + 1) * 128)
    h2 = _dot(_bf(gbuf[...]), _bf(w4[j]))
    res = habuf[t % 4, :, cs] + (x1buf[:, cs] + h2)
    outv[_rows(t * seg, seg), cs] = res.astype(outv.dtype)

  def st_out(t):
    r = _rows(t * seg, seg)
    pltpu.make_async_copy(outv.at[r], out_hbm.at[r], sems.at[7]).start()

  def step(s, do_r, do_b1, do_b2):
    t1, t2 = s - 1, s - 2
    ops = {}

    if do_r:
      fresh, probs = {}, {}
      lhs = st_lhs(s)

      def op_q(h):
        fresh[h] = [st_qkv(s, lhs, h, m) for m in range(3)]

      def op_s(h):
        probs[h] = st_scores(ld(s, h, 0, fresh[h][0]), ld(s, h, 1, fresh[h][1]))

      def op_p(h):
        st_pv(h, st_softmax(probs.pop(h)), ld(s, h, 2, fresh.pop(h)[2]))

      def op_xn(_):
        if isinstance(s, int):
          if s + 1 < nseg:
            st_xn(s + 1)
        else:
          st_xn(jnp.minimum(s + 1, nseg - 1))

      ops.update(Q=op_q, S=op_s, P=op_p, XN=op_xn, WO=lambda j: st_wo(s, j))

    if do_b1:
      ops.update(POST=lambda _: st_post(t1), B1=lambda j: st_b1(t1, j))

    if do_b2:
      ops.update(SHIFT=lambda _: st_shift(t2), B2=lambda j: st_b2(t2, j),
                 LN2=lambda _: st_ln2(t2), B3=lambda j: st_b3(t2, j),
                 B4=lambda j: st_b4(t2, j), OUT=lambda _: st_out(t2))

    for tok in SCHEDULE.split():
      name, _, rng = tok.partition(":")
      lo, hi = map(int, rng.split("-")) if rng else (0, 1)
      if name in ops:
        for i in range(lo, hi):
          ops[name](i)

  xb_cp.wait()
  for cp in strips("wo") + strips("w1"):
    cp.wait()
  st_xn(0)
  step(0, True, False, False)
  step(1, True, True, False)
  for cp in strips("w2") + strips("w3") + strips("w4"):
    cp.wait()

  def body(s, _):
    step(s, True, True, True)
    return 0

  lax.fori_loop(2, nseg, body, 0)
  step(nseg, False, True, True)
  step(nseg + 1, False, False, True)
  pltpu.make_async_copy(outv, out_hbm, sems.at[7]).wait()


def _forward(A_x, A_mem0, A_Wq, A_Wk, A_Wv, A_Wo, seg, B_w1, B_w2, B_w3, B_w4):
  assert A_x.shape == (1, S, D) and A_mem0.shape == (1, M, D)
  assert A_Wq.shape == (D, H, E) and A_Wo.shape == (H, E, D) and B_w3.shape == (D, F)
  assert seg == 32 and XP + (S // seg) * RX == S
  x2 = A_x.reshape(S, D)
  mem0 = A_mem0.reshape(M, D)
  wq, wk, wv = A_Wq, A_Wk, A_Wv
  wo = A_Wo.reshape(H * E, D)
  any_spec = pl.BlockSpec(memory_space=pl.ANY)
  scratch = [
      pltpu.VMEM((S, D), bf16),
      pltpu.VMEM((M, D), bf16),
      pltpu.VMEM((3 * H, D // 4, E), u32),
      pltpu.VMEM((3 * H, D // 4, E), u32),
      pltpu.VMEM((D // 128, H * E // 2, 128), u32),
      pltpu.VMEM((D // 128, D // 2, 128), u32),
      pltpu.VMEM((D // 128, D // 2, 128), u32),
      pltpu.VMEM((F // 128, D // 2, 128), u32),
      pltpu.VMEM((D // 128, F // 2, 128), u32),
      pltpu.VMEM((NSLOT, DCH, H // 2, E), u32),
      pltpu.VMEM((NCH, XP // 2, 128), u32),
      [pltpu.VMEM((3, RING, E), f32) for _ in range(H)],
      pltpu.VMEM((M, D), f32),
      pltpu.VMEM((2, RX, D), f32),
      pltpu.VMEM((M + seg, H * E), f32),
      pltpu.VMEM((seg, D), f32),
      pltpu.VMEM((4, seg, D), f32),
      pltpu.VMEM((4, seg, D), f32),
      pltpu.VMEM((S + 2 * PAD, D), f32),
      pltpu.VMEM((seg, D), f32),
      pltpu.VMEM((3, seg // 2, D), u32),
      pltpu.VMEM((seg // 2, F), u32),
      pltpu.VMEM((S, D), A_x.dtype),
      pltpu.SemaphoreType.DMA((NSLOT,)),
      pltpu.SemaphoreType.DMA((10,)),
  ]
  out = pl.pallas_call(
      functools.partial(_kernel, seg),
      out_shape=jax.ShapeDtypeStruct((S, D), A_x.dtype),
      in_specs=[any_spec] * 10,
      out_specs=any_spec,
      scratch_shapes=scratch,
      compiler_params=pltpu.CompilerParams(vmem_limit_bytes=126 * 2**20),
  )(x2, mem0, wq, wk, wv, wo, B_w1, B_w2, B_w3, B_w4)
  return out.reshape(1, S, D)


def pallas_sequential_preLN__memory_aug_recurrent_mem_tr__mixer_s_mlp__prompt_kernel(
    A_x, A_mem0, A_Wq, A_Wk, A_Wv, A_Wo, A_seg_len, B_x, B_w1, B_w2, B_w3, B_w4):
  del B_x
  return _forward(A_x, A_mem0, A_Wq, A_Wk, A_Wv, A_Wo, int(A_seg_len),
                  B_w1, B_w2, B_w3, B_w4)
```

```python
import functools

import jax
import jax.numpy as jnp
import numpy as np
from jax import lax
from jax.experimental import pallas as pl
from jax.experimental.pallas import tpu as pltpu

f32, bf16, u32 = jnp.float32, jnp.bfloat16, jnp.uint32

S, D, H, E, M, F = 2048, 1024, 32, 128, 8, 3584
LN_EPS = 1e-5
LOG2E = float(np.log2(np.e))
DCH = 128
NCH = D // DCH
NSLOT = 6
PAD = 8
XP = 512
PRB = 128
RX = 24
RING = 768
SCHEDULE = """
    POST Q:0-8 B1:0-8 Q:8-16 SHIFT B2:0-8 LN2 Q:16-24 B3:0-28 Q:24-32 XN
    B4:0-2 S:0-32 B4:2-5 P:0-32 B4:5-8 OUT WO:0-8
"""
DRAIN = """
    POST B1:0-8 SHIFTa B2a:0-8 SHIFTb B2b:0-8 LN2a B3a:0-28 LN2b B3b:0-28
    B4a:0-8 OUTa B4b:0-8 OUTb
"""
RING0 = 64


def _dot(a, b):
  return lax.dot_general(a, b, (((1,), (0,)), ((), ())), preferred_element_type=f32)


def _dot_nt(a, b):
  return lax.dot_general(a, b, (((1,), (1,)), ((), ())), preferred_element_type=f32)


def _bf(w):
  return pltpu.bitcast(w, bf16)


def _pk(x):
  return pltpu.bitcast(x.astype(bf16), u32)


def _ln(x):
  m = jnp.mean(x, axis=-1, keepdims=True)
  d = x - m
  v = jnp.mean(d * d, axis=-1, keepdims=True)
  return d * lax.rsqrt(v + LN_EPS)


def _gelu(x):
  c = np.float32(np.sqrt(2.0 / np.pi))
  inner = x * (c + (np.float32(c * 0.044715)) * (x * x))
  return (0.5 * x) * (1.0 + jnp.tanh(inner))


def _rows(i, n):
  if isinstance(i, int):
    return pl.ds(i, n)
  return pl.ds(pl.multiple_of(i, 8), n)


def _kernel(seg, x_hbm, mem0_hbm, wq_hbm, wk_hbm, wv_hbm, wo_hbm, w1_hbm, w2_hbm,
            w3_hbm, w4_hbm, out_hbm,
            xv, mem0v, wqa, wqb, wo, w1, w2, w3, w4, stage, xnp, qkvbuf, membuf, xnbuf,
            obuf, abuf, ybuf, habuf, h1buf, x1buf, zbuf, gbuf, outv, st_sem, sems):
  nseg = S // seg
  L = M + seg
  scale = np.float32(E ** -0.5)

  xa_cp = [pltpu.make_async_copy(x_hbm.at[r], xv.at[r], sems.at[k])
           for r, k in ((pl.ds(0, XP // 2), 0), (pl.ds(XP // 2, XP // 2), 9))]
  xb_cp = pltpu.make_async_copy(x_hbm.at[XP:S], xv.at[XP:S], sems.at[6])
  qkv_hbm = (wq_hbm, wk_hbm, wv_hbm)

  def stage_cp(m, c, slot):
    src = qkv_hbm[m].at[pl.ds(c * DCH, DCH)]
    return pltpu.make_async_copy(src, stage.at[slot].bitcast(bf16), st_sem.at[slot])

  def stage_wait(g):
    stage_cp(0, 0, g % NSLOT).wait()

  def stage_start(g):
    for m in range(3):
      if isinstance(g, int):
        if m * NCH <= g < (m + 1) * NCH:
          stage_cp(m, g - m * NCH, g % NSLOT).start()
      else:
        @pl.when((g >= m * NCH) & (g < (m + 1) * NCH))
        def _(m=m):
          stage_cp(m, g - m * NCH, g % NSLOT).start()

  strip_src = {"wo": (wo_hbm, wo, 1), "w1": (w1_hbm, w1, 2), "w2": (w2_hbm, w2, 3),
               "w3": (w3_hbm, w3, 4), "w4": (w4_hbm, w4, 5)}

  def strip(name, j):
    w_hbm, dst, sem = strip_src[name]
    col = j * 128 if isinstance(j, int) else pl.multiple_of(j * 128, 128)
    return pltpu.make_async_copy(
        w_hbm.at[:, pl.ds(col, 128)], dst.at[j].bitcast(bf16), sems.at[sem])

  def strips(name):
    return [strip(name, j) for j in range(strip_src[name][1].shape[0])]

  mem0_cp = pltpu.make_async_copy(mem0_hbm, mem0v, sems.at[8])
  mem0_cp.start()
  stage_start(0)
  h1buf[0:PAD, :] = jnp.zeros((PAD, D), f32)
  h1buf[PAD + S:PAD + S + PAD, :] = jnp.zeros((PAD, D), f32)

  mem0_cp.wait()
  membuf[...] = mem0v[...].astype(f32)
  for cp in xa_cp:
    cp.start()
  LNB = 64

  def ln_pro(half):
    xa_cp[half].wait()
    for i in range(half * XP // (2 * LNB), (half + 1) * XP // (2 * LNB)):
      xn = _pk(_ln(xv[pl.ds(i * LNB, LNB), :].astype(f32)))
      for kc in range(NCH):
        xnp[kc, pl.ds(i * (LNB // 2), LNB // 2), :] = xn[:, kc * 128:(kc + 1) * 128]

  def _pk_rows(g, off, n):
    return _rows(((g % NCH) // 2) * (DCH // 2) + off, n)

  NU = 2 * DCH // 16

  def relayout(g, wdst, units=range(NU)):
    for u in units:
      db, p = u // 2, u % 2
      v = _bf(stage[g % NSLOT, pl.ds(db * 16, 16), pl.ds(p * 8, 8), :])
      t = jnp.swapaxes(v, 0, 1)
      for k in range(16):
        wdst[(g // NCH) * H + p * 16 + k, _pk_rows(g, db * 8, 8), :] = (
            pltpu.bitcast(t[k], u32))

  def pro_dot(g, wsrc, may_be_first, b, h):
    m, kc = g // NCH, g % NCH
    rows = pl.ds(RING0 + b * PRB, PRB)
    part = _dot(_bf(xnp[kc, pl.ds(b * (PRB // 2), PRB // 2), :]),
                _bf(wsrc[m * H + h, _pk_rows(g, 0, DCH // 2), :]))
    dst = qkvbuf[h].at[m]
    old = dst[rows, :]
    if may_be_first:
      old = jnp.where(kc == 0, np.float32(0), old)
    dst[rows, :] = old + part

  NB = XP // PRB

  def pro_half(g, wsrc, half, may_be_first):
    for b in range(half * NB // 2, (half + 1) * NB // 2):
      for h in range(H):
        pro_dot(g, wsrc, may_be_first, b, h)

  NG = 3 * NCH
  def stage_wait_if(g):
    pl.when(g < NG)(lambda: stage_wait(g))

  stage_wait(0)
  for g in range(1, NSLOT):
    stage_start(g)
  relayout(0, wqa)
  stage_start(NSLOT)
  ln_pro(0)
  ln_pro(1)
  pro_half(0, wqa, 0, True)
  pro_half(0, wqa, 1, True)
  stage_wait(1)
  relayout(1, wqb)
  stage_start(NSLOT + 1)
  pro_half(1, wqb, 0, False)
  stage_wait(2)
  stage_wait(3)

  def pro_body(i, _):
    g = 2 * i + 1
    pro_half(g, wqb, 1, False)
    relayout(g + 1, wqa)
    pro_half(g + 1, wqa, 0, True)
    pro_half(g + 1, wqa, 1, True)
    relayout(g + 2, wqb)
    pro_half(g + 2, wqb, 0, False)
    stage_start(g + NSLOT + 1)
    stage_start(g + NSLOT + 2)

    @pl.when(i < 8)
    def _():
      for name, j in (("wo", i), ("w1", i), ("w2", i), ("w3", 2 * i), ("w3", 2 * i + 1)):
        strip(name, j).start()

    @pl.when(i == 8)
    def _():
      xb_cp.start()
      for j in range(16, 24):
        strip("w3", j).start()

    @pl.when(i == 9)
    def _():
      for j in range(24, 28):
        strip("w3", j).start()
      for j in range(4):
        strip("w4", j).start()

    @pl.when(i == 10)
    def _():
      for j in range(4, 8):
        strip("w4", j).start()

    stage_wait_if(g + 3)
    stage_wait_if(g + 4)
    return 0

  lax.fori_loop(0, NG // 2 - 1, pro_body, 0)

  def late_pro(k):
    b = NB // 2 + k
    return lambda j: [pro_dot(NG - 1, wqb, False, b, h) for h in range(j * 4, j * 4 + 4)]

  row = lax.broadcasted_iota(jnp.int32, (L, L), 0)
  col = lax.broadcasted_iota(jnp.int32, (L, L), 1)
  mask = (row < M) | (col <= row)

  def st_xn(s):
    xs = xv[_rows(XP + s * RX, RX), :].astype(f32)
    xnbuf[s % 2] = _ln(xs)

  def wrow(s):
    return _rows(((s + (XP + RING0) // RX) % (RING // RX)) * RX, RX)

  def rrow(s):
    return _rows(((s + RING0 // seg) % (RING // seg)) * seg, seg)

  def st_lhs(s):
    return jnp.concatenate([membuf[...], xnbuf[s % 2]], axis=0).astype(bf16)

  def st_qkv(s, lhs, h, m):
    half = DCH // 2
    w = jnp.concatenate(
        [(wqa, wqb)[kc % 2][m * H + h, pl.ds((kc // 2) * half, half), :]
         for kc in range(NCH)], axis=0)
    r = _dot(lhs, _bf(w))
    qkvbuf[h][m, wrow(s), :] = r[M:]
    return r[:M]

  def ld(s, h, m, fresh):
    return jnp.concatenate([fresh, qkvbuf[h][m, rrow(s), :]], axis=0)

  def st_scores(q, k):
    return _dot_nt(q, k.astype(bf16))

  def st_softmax(sc):
    t = jnp.where(mask, sc * np.float32(scale * LOG2E), np.float32(-1e9 * LOG2E))
    e = jnp.exp2(t - jnp.max(t, axis=-1, keepdims=True))
    l = jnp.sum(e, axis=-1, keepdims=True)
    r = pl.reciprocal(l, approx=True)
    r = r * (2.0 - l * r)
    return e * r

  def st_pv(h, p, v):
    obuf[:, h * E:(h + 1) * E] = _dot(p, v.astype(bf16))

  def st_wo(s, j):
    r = _dot(obuf[...], _bf(wo[j]))
    membuf[:, j * 128:(j + 1) * 128] = r[:M]
    abuf[:, j * 128:(j + 1) * 128] = r[M:]

  def st_post(t):
    xs = xv[_rows(t * seg, seg), :].astype(f32)
    ha = xs + abuf[...]
    habuf[t % 4] = ha
    y = _ln(ha)
    ybuf[t % 4] = y
    zbuf[0] = _pk(_ln(y))

  def st_b1(t, j):
    g = _gelu(_dot(_bf(zbuf[0]), _bf(w1[j])))
    h1buf[_rows(PAD + t * seg, seg), j * 128:(j + 1) * 128] = g

  c4 = D // 4

  def st_shift(t, u):
    win = h1buf[_rows(t * seg, seg + 2 * PAD), :]
    g0 = win[PAD - 1:PAD - 1 + seg, 0 * c4:1 * c4]
    g1 = win[PAD + 1:PAD + 1 + seg, 1 * c4:2 * c4]
    g2 = win[PAD - 2:PAD - 2 + seg, 2 * c4:3 * c4]
    g3 = win[PAD + 2:PAD + 2 + seg, 3 * c4:4 * c4]
    zbuf[1 + 2 * u] = _pk(jnp.concatenate([g0, g1, g2, g3], axis=1))

  def st_b2(t, u, j):
    cs = slice(j * 128, (j + 1) * 128)
    x1buf[u, :, cs] = ybuf[t % 4, :, cs] + _dot(_bf(zbuf[1 + 2 * u]), _bf(w2[j]))

  def st_ln2(t, u):
    zbuf[2 + 2 * u] = _pk(_ln(x1buf[u]))

  def st_b3(t, u, j):
    gbuf[u, :, j * 128:(j + 1) * 128] = _pk(_gelu(_dot(_bf(zbuf[2 + 2 * u]), _bf(w3[j]))))

  def st_b4(t, u, j):
    cs = slice(j * 128, (j + 1) * 128)
    h2 = _dot(_bf(gbuf[u]), _bf(w4[j]))
    res = habuf[t % 4, :, cs] + (x1buf[u, :, cs] + h2)
    outv[_rows(t * seg, seg), cs] = res.astype(outv.dtype)

  def st_out(t):
    r = _rows(t * seg, seg)
    pltpu.make_async_copy(outv.at[r], out_hbm.at[r], sems.at[7]).start()

  def b_ops(t, u, suffix=""):
    ops = dict(SHIFT=lambda _: st_shift(t, u), B2=lambda j: st_b2(t, u, j),
               LN2=lambda _: st_ln2(t, u), B3=lambda j: st_b3(t, u, j),
               B4=lambda j: st_b4(t, u, j), OUT=lambda _: st_out(t))
    return {k + suffix: v for k, v in ops.items()}

  def run(schedule, ops):
    for tok in schedule.split():
      name, _, rng = tok.partition(":")
      lo, hi = map(int, rng.split("-")) if rng else (0, 1)
      if name in ops:
        for i in range(lo, hi):
          ops[name](i)

  def step(s, do_b1, do_b2, filler=None):
    t1, t2 = s - 1, s - 2
    ops = {}

    fresh, probs = {}, {}
    lhs = st_lhs(s)

    def op_q(h):
      fresh[h] = [st_qkv(s, lhs, h, m) for m in range(3)]

    def op_s(h):
      probs[h] = st_scores(ld(s, h, 0, fresh[h][0]), ld(s, h, 1, fresh[h][1]))

    def op_p(h):
      st_pv(h, st_softmax(probs.pop(h)), ld(s, h, 2, fresh.pop(h)[2]))

    def op_xn(_):
      st_xn(s + 1 if isinstance(s, int) else jnp.minimum(s + 1, nseg - 1))

    ops.update(Q=op_q, S=op_s, P=op_p, XN=op_xn, WO=lambda j: st_wo(s, j))

    if do_b1:
      ops.update(POST=lambda _: st_post(t1), B1=lambda j: st_b1(t1, j))

    if do_b2:
      ops.update(b_ops(t2, 0))
    elif filler is not None:
      ops.update(B4=filler)

    run(SCHEDULE, ops)

  xb_cp.wait()
  for cp in strips("wo") + strips("w1"):
    cp.wait()
  st_xn(0)
  assert NB == 4
  step(0, False, False, late_pro(0))
  step(1, True, False, late_pro(1))
  for cp in strips("w2") + strips("w3") + strips("w4"):
    cp.wait()

  def body(s, _):
    step(s, True, True)
    return 0

  lax.fori_loop(2, nseg, body, 0)
  t = nseg - 1
  ops = dict(POST=lambda _: st_post(t), B1=lambda j: st_b1(t, j))
  ops.update(b_ops(t - 1, 0, "a"))
  ops.update(b_ops(t, 1, "b"))
  run(DRAIN, ops)
  pltpu.make_async_copy(outv, out_hbm, sems.at[7]).wait()


def _forward(A_x, A_mem0, A_Wq, A_Wk, A_Wv, A_Wo, seg, B_w1, B_w2, B_w3, B_w4):
  assert A_x.shape == (1, S, D) and A_mem0.shape == (1, M, D)
  assert A_Wq.shape == (D, H, E) and A_Wo.shape == (H, E, D) and B_w3.shape == (D, F)
  assert seg == 32 and XP + (S // seg) * RX == S
  x2 = A_x.reshape(S, D)
  mem0 = A_mem0.reshape(M, D)
  wq, wk, wv = A_Wq, A_Wk, A_Wv
  wo = A_Wo.reshape(H * E, D)
  any_spec = pl.BlockSpec(memory_space=pl.ANY)
  scratch = [
      pltpu.VMEM((S, D), bf16),
      pltpu.VMEM((M, D), bf16),
      pltpu.VMEM((3 * H, D // 4, E), u32),
      pltpu.VMEM((3 * H, D // 4, E), u32),
      pltpu.VMEM((D // 128, H * E // 2, 128), u32),
      pltpu.VMEM((D // 128, D // 2, 128), u32),
      pltpu.VMEM((D // 128, D // 2, 128), u32),
      pltpu.VMEM((F // 128, D // 2, 128), u32),
      pltpu.VMEM((D // 128, F // 2, 128), u32),
      pltpu.VMEM((NSLOT, DCH, H // 2, E), u32),
      pltpu.VMEM((NCH, XP // 2, 128), u32),
      [pltpu.VMEM((3, RING, E), f32) for _ in range(H)],
      pltpu.VMEM((M, D), f32),
      pltpu.VMEM((2, RX, D), f32),
      pltpu.VMEM((M + seg, H * E), f32),
      pltpu.VMEM((seg, D), f32),
      pltpu.VMEM((4, seg, D), f32),
      pltpu.VMEM((4, seg, D), f32),
      pltpu.VMEM((S + 2 * PAD, D), f32),
      pltpu.VMEM((2, seg, D), f32),
      pltpu.VMEM((5, seg // 2, D), u32),
      pltpu.VMEM((2, seg // 2, F), u32),
      pltpu.VMEM((S, D), A_x.dtype),
      pltpu.SemaphoreType.DMA((NSLOT,)),
      pltpu.SemaphoreType.DMA((10,)),
  ]
  out = pl.pallas_call(
      functools.partial(_kernel, seg),
      out_shape=jax.ShapeDtypeStruct((S, D), A_x.dtype),
      in_specs=[any_spec] * 10,
      out_specs=any_spec,
      scratch_shapes=scratch,
      compiler_params=pltpu.CompilerParams(vmem_limit_bytes=126 * 2**20),
  )(x2, mem0, wq, wk, wv, wo, B_w1, B_w2, B_w3, B_w4)
  return out.reshape(1, S, D)


def pallas_sequential_preLN__memory_aug_recurrent_mem_tr__mixer_s_mlp__prompt_kernel(
    A_x, A_mem0, A_Wq, A_Wk, A_Wv, A_Wo, A_seg_len, B_x, B_w1, B_w2, B_w3, B_w4):
  del B_x
  return _forward(A_x, A_mem0, A_Wq, A_Wk, A_Wv, A_Wo, int(A_seg_len),
                  B_w1, B_w2, B_w3, B_w4)
```

```python
import functools

import jax
import jax.numpy as jnp
import numpy as np
from jax import lax
from jax.experimental import pallas as pl
from jax.experimental.pallas import tpu as pltpu

f32, bf16, u32 = jnp.float32, jnp.bfloat16, jnp.uint32

S, D, H, E, M, F = 2048, 1024, 32, 128, 8, 3584
LN_EPS = 1e-5
LOG2E = float(np.log2(np.e))
DCH = 128
NCH = D // DCH
NSLOT = 6
PAD = 8
XP = 512
PRB = 128
RX = 24
RING = 768
RING0 = 64
SEG = 32

SCHEDULE = """
    POST Q:0-8 B1:0-8 Q:8-16 SHIFT B2:0-8 LN2 Q:16-24 B3:0-28 Q:24-32 XN
    B4:0-2 S:0-32 B4:2-5 P:0-32 B4:5-8 OUT WO:0-8
"""
DRAIN = """
    POST B1:0-8 SHIFTa B2a:0-8 SHIFTb B2b:0-8 LN2a B3a:0-28 LN2b B3b:0-28
    B4a:0-8 OUTa B4b:0-8 OUTb
"""


def _dot(a, b):
  return lax.dot_general(a, b, (((1,), (0,)), ((), ())), preferred_element_type=f32)


def _dot_nt(a, b):
  return lax.dot_general(a, b, (((1,), (1,)), ((), ())), preferred_element_type=f32)


def _bf(w):
  return pltpu.bitcast(w, bf16)


def _pk(x):
  return pltpu.bitcast(x.astype(bf16), u32)


def _ln(x):
  m = jnp.mean(x, axis=-1, keepdims=True)
  d = x - m
  v = jnp.mean(d * d, axis=-1, keepdims=True)
  return d * lax.rsqrt(v + LN_EPS)


def _gelu(x):
  c = np.float32(np.sqrt(2.0 / np.pi))
  inner = x * (c + (np.float32(c * 0.044715)) * (x * x))
  return (0.5 * x) * (1.0 + jnp.tanh(inner))


def _rows(i, n):
  if isinstance(i, int):
    return pl.ds(i, n)
  return pl.ds(pl.multiple_of(i, 8), n)


def _kernel(seg, x_hbm, mem0_hbm, wq_hbm, wk_hbm, wv_hbm, wo_hbm, w1_hbm, w2_hbm,
            w3_hbm, w4_hbm, out_hbm,
            xv, mem0v, wqa, wqb, wo, w1, w2, w3, w4, stage, xnp, qkvbuf, membuf, xnbuf,
            obuf, abuf, ybuf, habuf, h1buf, x1buf, zbuf, gbuf, outv, st_sem, sems):
  nseg = S // seg
  L = M + seg
  scale = np.float32(E ** -0.5)

  xa_cp = [pltpu.make_async_copy(x_hbm.at[r], xv.at[r], sems.at[k])
           for r, k in ((pl.ds(0, XP // 2), 0), (pl.ds(XP // 2, XP // 2), 9))]
  xb_cp = pltpu.make_async_copy(x_hbm.at[XP:S], xv.at[XP:S], sems.at[6])
  qkv_hbm = (wq_hbm, wk_hbm, wv_hbm)

  def stage_cp(m, c, slot):
    src = qkv_hbm[m].at[pl.ds(c * DCH, DCH)]
    return pltpu.make_async_copy(src, stage.at[slot].bitcast(bf16), st_sem.at[slot])

  def stage_wait(g):
    stage_cp(0, 0, g % NSLOT).wait()

  def stage_start(g):
    for m in range(3):
      if isinstance(g, int):
        if m * NCH <= g < (m + 1) * NCH:
          stage_cp(m, g - m * NCH, g % NSLOT).start()
      else:
        @pl.when((g >= m * NCH) & (g < (m + 1) * NCH))
        def _(m=m):
          stage_cp(m, g - m * NCH, g % NSLOT).start()

  strip_src = {"wo": (wo_hbm, wo, 1), "w1": (w1_hbm, w1, 2), "w2": (w2_hbm, w2, 3),
               "w3": (w3_hbm, w3, 4), "w4": (w4_hbm, w4, 5)}

  def strip(name, j):
    w_hbm, dst, sem = strip_src[name]
    col = j * 128 if isinstance(j, int) else pl.multiple_of(j * 128, 128)
    return pltpu.make_async_copy(
        w_hbm.at[:, pl.ds(col, 128)], dst.at[j].bitcast(bf16), sems.at[sem])

  def strips(name):
    return [strip(name, j) for j in range(strip_src[name][1].shape[0])]

  mem0_cp = pltpu.make_async_copy(mem0_hbm, mem0v, sems.at[8])
  mem0_cp.start()
  stage_start(0)
  h1buf[0:PAD, :] = jnp.zeros((PAD, D), f32)
  h1buf[PAD + S:PAD + S + PAD, :] = jnp.zeros((PAD, D), f32)

  mem0_cp.wait()
  membuf[...] = mem0v[...].astype(f32)
  for cp in xa_cp:
    cp.start()
  LNB = 64

  def ln_pro(half):
    xa_cp[half].wait()
    for i in range(half * XP // (2 * LNB), (half + 1) * XP // (2 * LNB)):
      xn = _pk(_ln(xv[pl.ds(i * LNB, LNB), :].astype(f32)))
      for kc in range(NCH):
        xnp[kc, pl.ds(i * (LNB // 2), LNB // 2), :] = xn[:, kc * 128:(kc + 1) * 128]

  def _pk_rows(g, off, n):
    return _rows(((g % NCH) // 2) * (DCH // 2) + off, n)

  NU = 2 * DCH // 16

  def relayout(g, wdst, units=range(NU)):
    for u in units:
      db, p = u // 2, u % 2
      v = _bf(stage[g % NSLOT, pl.ds(db * 16, 16), pl.ds(p * 8, 8), :])
      t = jnp.swapaxes(v, 0, 1)
      for k in range(16):
        wdst[(g // NCH) * H + p * 16 + k, _pk_rows(g, db * 8, 8), :] = (
            pltpu.bitcast(t[k], u32))

  def pro_dot(g, wsrc, may_be_first, b, h):
    m, kc = g // NCH, g % NCH
    rows = pl.ds(RING0 + b * PRB, PRB)
    part = _dot(_bf(xnp[kc, pl.ds(b * (PRB // 2), PRB // 2), :]),
                _bf(wsrc[m * H + h, _pk_rows(g, 0, DCH // 2), :]))
    dst = qkvbuf[h].at[m]
    if may_be_first and isinstance(g, int):
      dst[rows, :] = part if kc == 0 else dst[rows, :] + part
      return
    old = dst[rows, :]
    if may_be_first:
      old = jnp.where(kc == 0, np.float32(0), old)
    dst[rows, :] = old + part

  NB = XP // PRB

  def pro_half(g, wsrc, half, may_be_first):
    for b in range(half * NB // 2, (half + 1) * NB // 2):
      for h in range(H):
        pro_dot(g, wsrc, may_be_first, b, h)

  NG = 3 * NCH

  def stage_wait_if(g):
    pl.when(g < NG)(lambda: stage_wait(g))

  stage_wait(0)
  for g in range(1, NSLOT):
    stage_start(g)
  relayout(0, wqa)
  stage_start(NSLOT)
  ln_pro(0)
  ln_pro(1)
  pro_half(0, wqa, 0, True)
  pro_half(0, wqa, 1, True)
  stage_wait(1)
  relayout(1, wqb)
  stage_start(NSLOT + 1)
  pro_half(1, wqb, 0, False)
  stage_wait(2)
  stage_wait(3)

  def pro_body(i, _):
    g = 2 * i + 1
    pro_half(g, wqb, 1, False)
    relayout(g + 1, wqa)
    pro_half(g + 1, wqa, 0, True)
    pro_half(g + 1, wqa, 1, True)
    relayout(g + 2, wqb)
    pro_half(g + 2, wqb, 0, False)
    stage_start(g + NSLOT + 1)
    stage_start(g + NSLOT + 2)

    @pl.when(i < 8)
    def _():
      for name, j in (("wo", i), ("w1", i), ("w2", i), ("w3", 2 * i), ("w3", 2 * i + 1)):
        strip(name, j).start()

    @pl.when(i == 8)
    def _():
      xb_cp.start()
      for j in range(16, 24):
        strip("w3", j).start()

    @pl.when(i == 9)
    def _():
      for j in range(24, 28):
        strip("w3", j).start()
      for j in range(4):
        strip("w4", j).start()

    @pl.when(i == 10)
    def _():
      for j in range(4, 8):
        strip("w4", j).start()

    stage_wait_if(g + 3)
    stage_wait_if(g + 4)
    return 0

  lax.fori_loop(0, NG // 2 - 1, pro_body, 0)

  def late_pro(k):
    b = NB // 2 + k
    return lambda j: [pro_dot(NG - 1, wqb, False, b, h) for h in range(j * 4, j * 4 + 4)]

  row = lax.broadcasted_iota(jnp.int32, (L, L), 0)
  col = lax.broadcasted_iota(jnp.int32, (L, L), 1)
  mask = (row < M) | (col <= row)

  def st_xn(s):
    xs = xv[_rows(XP + s * RX, RX), :].astype(f32)
    xnbuf[s % 2] = _ln(xs)

  def wrow(s):
    return _rows(((s + (XP + RING0) // RX) % (RING // RX)) * RX, RX)

  def rrow(s):
    return _rows(((s + RING0 // seg) % (RING // seg)) * seg, seg)

  def st_lhs(s):
    return jnp.concatenate([membuf[...], xnbuf[s % 2]], axis=0).astype(bf16)

  def st_qkv(s, lhs, h, m):
    half = DCH // 2
    w = jnp.concatenate(
        [(wqa, wqb)[kc % 2][m * H + h, pl.ds((kc // 2) * half, half), :]
         for kc in range(NCH)], axis=0)
    r = _dot(lhs, _bf(w))
    qkvbuf[h][m, wrow(s), :] = r[M:]
    return r[:M]

  def ld(s, h, m, fresh):
    return jnp.concatenate([fresh, qkvbuf[h][m, rrow(s), :]], axis=0)

  def st_scores(q, k):
    return _dot_nt(q, k.astype(bf16))

  def st_softmax(sc):
    t = jnp.where(mask, sc * np.float32(scale * LOG2E), np.float32(-1e9 * LOG2E))
    e = jnp.exp2(t - jnp.max(t, axis=-1, keepdims=True))
    l = jnp.sum(e, axis=-1, keepdims=True)
    r = pl.reciprocal(l, approx=True)
    r = r * (2.0 - l * r)
    return e * r

  def st_pv(h, p, v):
    obuf[:, h * E:(h + 1) * E] = _dot(p, v.astype(bf16))

  def st_wo(s, j):
    r = _dot(obuf[...], _bf(wo[j]))
    membuf[:, j * 128:(j + 1) * 128] = r[:M]
    abuf[:, j * 128:(j + 1) * 128] = r[M:]

  def st_post(t):
    xs = xv[_rows(t * seg, seg), :].astype(f32)
    ha = xs + abuf[...]
    habuf[t % 4] = ha
    y = _ln(ha)
    ybuf[t % 4] = y
    zbuf[0] = _pk(_ln(y))

  def st_b1(t, j):
    g = _gelu(_dot(_bf(zbuf[0]), _bf(w1[j])))
    h1buf[_rows(PAD + t * seg, seg), j * 128:(j + 1) * 128] = g

  c4 = D // 4

  def st_shift(t, u):
    win = h1buf[_rows(t * seg, seg + 2 * PAD), :]
    g0 = win[PAD - 1:PAD - 1 + seg, 0 * c4:1 * c4]
    g1 = win[PAD + 1:PAD + 1 + seg, 1 * c4:2 * c4]
    g2 = win[PAD - 2:PAD - 2 + seg, 2 * c4:3 * c4]
    g3 = win[PAD + 2:PAD + 2 + seg, 3 * c4:4 * c4]
    zbuf[1 + 2 * u] = _pk(jnp.concatenate([g0, g1, g2, g3], axis=1))

  def st_b2(t, u, j):
    cs = slice(j * 128, (j + 1) * 128)
    x1buf[u, :, cs] = ybuf[t % 4, :, cs] + _dot(_bf(zbuf[1 + 2 * u]), _bf(w2[j]))

  def st_ln2(t, u):
    zbuf[2 + 2 * u] = _pk(_ln(x1buf[u]))

  def st_b3(t, u, j):
    gbuf[u, :, j * 128:(j + 1) * 128] = _pk(_gelu(_dot(_bf(zbuf[2 + 2 * u]), _bf(w3[j]))))

  def st_b4(t, u, j):
    cs = slice(j * 128, (j + 1) * 128)
    h2 = _dot(_bf(gbuf[u]), _bf(w4[j]))
    res = habuf[t % 4, :, cs] + (x1buf[u, :, cs] + h2)
    outv[_rows(t * seg, seg), cs] = res.astype(outv.dtype)

  def st_out(t):
    r = _rows(t * seg, seg)
    pltpu.make_async_copy(outv.at[r], out_hbm.at[r], sems.at[7]).start()

  def b_ops(t, u, suffix=""):
    ops = dict(SHIFT=lambda _: st_shift(t, u), B2=lambda j: st_b2(t, u, j),
               LN2=lambda _: st_ln2(t, u), B3=lambda j: st_b3(t, u, j),
               B4=lambda j: st_b4(t, u, j), OUT=lambda _: st_out(t))
    return {k + suffix: v for k, v in ops.items()}

  def run(schedule, ops):
    for tok in schedule.split():
      name, _, rng = tok.partition(":")
      lo, hi = map(int, rng.split("-")) if rng else (0, 1)
      if name in ops:
        for i in range(lo, hi):
          ops[name](i)

  def step(s, do_b1, do_b2, filler=None):
    t1, t2 = s - 1, s - 2
    ops = {}

    fresh, probs = {}, {}
    lhs = st_lhs(s)

    def op_q(h):
      fresh[h] = [st_qkv(s, lhs, h, m) for m in range(3)]

    def op_s(h):
      probs[h] = st_scores(ld(s, h, 0, fresh[h][0]), ld(s, h, 1, fresh[h][1]))

    def op_p(h):
      st_pv(h, st_softmax(probs.pop(h)), ld(s, h, 2, fresh.pop(h)[2]))

    def op_xn(_):
      st_xn(s + 1 if isinstance(s, int) else jnp.minimum(s + 1, nseg - 1))

    ops.update(Q=op_q, S=op_s, P=op_p, XN=op_xn, WO=lambda j: st_wo(s, j))

    if do_b1:
      ops.update(POST=lambda _: st_post(t1), B1=lambda j: st_b1(t1, j))

    if do_b2:
      ops.update(b_ops(t2, 0))
    elif filler is not None:
      ops.update(B4=filler)

    run(SCHEDULE, ops)

  xb_cp.wait()
  for cp in strips("wo") + strips("w1"):
    cp.wait()
  st_xn(0)
  assert NB == 4
  step(0, False, False, late_pro(0))
  step(1, True, False, late_pro(1))
  for cp in strips("w2") + strips("w3") + strips("w4"):
    cp.wait()

  def body(s, _):
    step(s, True, True)
    return 0

  lax.fori_loop(2, nseg, body, 0)
  t = nseg - 1
  ops = dict(POST=lambda _: st_post(t), B1=lambda j: st_b1(t, j))
  ops.update(b_ops(t - 1, 0, "a"))
  ops.update(b_ops(t, 1, "b"))
  run(DRAIN, ops)
  pltpu.make_async_copy(outv, out_hbm, sems.at[7]).wait()


def _forward(A_x, A_mem0, A_Wq, A_Wk, A_Wv, A_Wo, seg, B_w1, B_w2, B_w3, B_w4):
  assert A_x.shape == (1, S, D) and A_mem0.shape == (1, M, D)
  assert A_Wq.shape == (D, H, E) and A_Wo.shape == (H, E, D) and B_w3.shape == (D, F)
  assert seg == SEG and XP + (S // seg) * RX == S
  x2 = A_x.reshape(S, D)
  mem0 = A_mem0.reshape(M, D)
  wq, wk, wv = A_Wq, A_Wk, A_Wv
  wo = A_Wo.reshape(H * E, D)
  any_spec = pl.BlockSpec(memory_space=pl.ANY)
  scratch = [
      pltpu.VMEM((S, D), bf16),
      pltpu.VMEM((M, D), bf16),
      pltpu.VMEM((3 * H, D // 4, E), u32),
      pltpu.VMEM((3 * H, D // 4, E), u32),
      pltpu.VMEM((D // 128, H * E // 2, 128), u32),
      pltpu.VMEM((D // 128, D // 2, 128), u32),
      pltpu.VMEM((D // 128, D // 2, 128), u32),
      pltpu.VMEM((F // 128, D // 2, 128), u32),
      pltpu.VMEM((D // 128, F // 2, 128), u32),
      pltpu.VMEM((NSLOT, DCH, H // 2, E), u32),
      pltpu.VMEM((NCH, XP // 2, 128), u32),
      [pltpu.VMEM((3, RING, E), f32) for _ in range(H)],
      pltpu.VMEM((M, D), f32),
      pltpu.VMEM((2, RX, D), f32),
      pltpu.VMEM((M + seg, H * E), f32),
      pltpu.VMEM((seg, D), f32),
      pltpu.VMEM((4, seg, D), f32),
      pltpu.VMEM((4, seg, D), f32),
      pltpu.VMEM((S + 2 * PAD, D), f32),
      pltpu.VMEM((2, seg, D), f32),
      pltpu.VMEM((5, seg // 2, D), u32),
      pltpu.VMEM((2, seg // 2, F), u32),
      pltpu.VMEM((S, D), A_x.dtype),
      pltpu.SemaphoreType.DMA((NSLOT,)),
      pltpu.SemaphoreType.DMA((10,)),
  ]
  out = pl.pallas_call(
      functools.partial(_kernel, seg),
      out_shape=jax.ShapeDtypeStruct((S, D), A_x.dtype),
      in_specs=[any_spec] * 10,
      out_specs=any_spec,
      scratch_shapes=scratch,
      compiler_params=pltpu.CompilerParams(vmem_limit_bytes=126 * 2**20),
  )(x2, mem0, wq, wk, wv, wo, B_w1, B_w2, B_w3, B_w4)
  return out.reshape(1, S, D)


def pallas_sequential_preLN__memory_aug_recurrent_mem_tr__mixer_s_mlp__prompt_kernel(
    A_x, A_mem0, A_Wq, A_Wk, A_Wv, A_Wo, A_seg_len, B_x, B_w1, B_w2, B_w3, B_w4):
  del B_x
  seg = int(A_seg_len) if isinstance(A_seg_len, (int, np.integer)) else SEG
  return _forward(A_x, A_mem0, A_Wq, A_Wk, A_Wv, A_Wo, seg, B_w1, B_w2, B_w3, B_w4)
```

```python
import functools

import jax
import jax.numpy as jnp
import numpy as np
from jax import lax
from jax.experimental import pallas as pl
from jax.experimental.pallas import tpu as pltpu

f32, bf16, u32 = jnp.float32, jnp.bfloat16, jnp.uint32

S, D, H, E, M, F = 2048, 1024, 32, 128, 8, 3584
LN_EPS = 1e-5
LOG2E = float(np.log2(np.e))
DCH = 128
NCH = D // DCH
NSLOT = 6
PAD = 8
XP = 512
PRB = 128
RX = 24
RING = 768
RING0 = 64
SEG = 32

SCHEDULE = """
    POST Q:0-8 B1:0-8 Q:8-16 SHIFT B2:0-8 LN2 Q:16-24 B3:0-28 Q:24-32 XN
    B4:0-2 S:0-32 B4:2-5 P:0-32 B4:5-8 OUT WO:0-8
"""
DRAIN = """
    POST B1:0-8 SHIFTa B2a:0-8 SHIFTb B2b:0-8 LN2a B3a:0-28 LN2b B3b:0-28
    B4a:0-8 OUTa B4b:0-8 OUTb
"""


def _dot(a, b):
  return lax.dot_general(a, b, (((1,), (0,)), ((), ())), preferred_element_type=f32)


def _dot_nt(a, b):
  return lax.dot_general(a, b, (((1,), (1,)), ((), ())), preferred_element_type=f32)


def _bf(w):
  return pltpu.bitcast(w, bf16)


def _pk(x):
  return pltpu.bitcast(x.astype(bf16), u32)


def _ln(x):
  m = jnp.mean(x, axis=-1, keepdims=True)
  d = x - m
  v = jnp.mean(d * d, axis=-1, keepdims=True)
  return d * lax.rsqrt(v + LN_EPS)


def _gelu(x):
  c = np.float32(np.sqrt(2.0 / np.pi))
  inner = x * (c + (np.float32(c * 0.044715)) * (x * x))
  return (0.5 * x) * (1.0 + jnp.tanh(inner))


def _rows(i, n):
  if isinstance(i, int):
    return pl.ds(i, n)
  return pl.ds(pl.multiple_of(i, 8), n)


def _kernel(seg, x_hbm, mem0_hbm, wq_hbm, wk_hbm, wv_hbm, wo_hbm, w1_hbm, w2_hbm,
            w3_hbm, w4_hbm, out_hbm,
            xv, mem0v, wqa, wqb, wo, w1, w2, w3, w4, stage, xnp, qkvbuf, membuf, xnbuf,
            obuf, abuf, ybuf, habuf, h1buf, x1buf, zbuf, gbuf, outv, st_sem, sems):
  nseg = S // seg
  L = M + seg
  scale = np.float32(E ** -0.5)

  xa_cp = [pltpu.make_async_copy(x_hbm.at[pl.ds(b * PRB, PRB)],
                                 xv.at[pl.ds(b * PRB, PRB)], sems.at[k])
           for b, k in enumerate((0, 9, 10, 11))]
  xb_cp = pltpu.make_async_copy(x_hbm.at[XP:S], xv.at[XP:S], sems.at[6])
  qkv_hbm = (wq_hbm, wk_hbm, wv_hbm)

  def stage_cp(m, c, slot):
    src = qkv_hbm[m].at[pl.ds(c * DCH, DCH)]
    return pltpu.make_async_copy(src, stage.at[slot].bitcast(bf16), st_sem.at[slot])

  def stage_wait(g):
    stage_cp(0, 0, g % NSLOT).wait()

  def stage_start(g):
    for m in range(3):
      if isinstance(g, int):
        if m * NCH <= g < (m + 1) * NCH:
          stage_cp(m, g - m * NCH, g % NSLOT).start()
      else:
        @pl.when((g >= m * NCH) & (g < (m + 1) * NCH))
        def _(m=m):
          stage_cp(m, g - m * NCH, g % NSLOT).start()

  strip_src = {"wo": (wo_hbm, wo, 1), "w1": (w1_hbm, w1, 2), "w2": (w2_hbm, w2, 3),
               "w3": (w3_hbm, w3, 4), "w4": (w4_hbm, w4, 5)}

  def strip(name, j):
    w_hbm, dst, sem = strip_src[name]
    col = j * 128 if isinstance(j, int) else pl.multiple_of(j * 128, 128)
    return pltpu.make_async_copy(
        w_hbm.at[:, pl.ds(col, 128)], dst.at[j].bitcast(bf16), sems.at[sem])

  def strips(name):
    return [strip(name, j) for j in range(strip_src[name][1].shape[0])]

  mem0_cp = pltpu.make_async_copy(mem0_hbm, mem0v, sems.at[8])
  mem0_cp.start()
  stage_start(0)
  h1buf[0:PAD, :] = jnp.zeros((PAD, D), f32)
  h1buf[PAD + S:PAD + S + PAD, :] = jnp.zeros((PAD, D), f32)

  mem0_cp.wait()
  membuf[...] = mem0v[...].astype(f32)
  for cp in xa_cp:
    cp.start()
  LNB = 64

  def ln_pro(b):
    xa_cp[b].wait()
    for i in range(b * PRB // LNB, (b + 1) * PRB // LNB):
      xn = _pk(_ln(xv[pl.ds(i * LNB, LNB), :].astype(f32)))
      for kc in range(NCH):
        xnp[kc, pl.ds(i * (LNB // 2), LNB // 2), :] = xn[:, kc * 128:(kc + 1) * 128]

  def _pk_rows(g, off, n):
    return _rows(((g % NCH) // 2) * (DCH // 2) + off, n)

  NU = 2 * DCH // 16

  def relayout(g, wdst, units=range(NU)):
    for u in units:
      db, p = u // 2, u % 2
      v = _bf(stage[g % NSLOT, pl.ds(db * 16, 16), pl.ds(p * 8, 8), :])
      t = jnp.swapaxes(v, 0, 1)
      for k in range(16):
        wdst[(g // NCH) * H + p * 16 + k, _pk_rows(g, db * 8, 8), :] = (
            pltpu.bitcast(t[k], u32))

  def pro_dot(g, wsrc, may_be_first, b, h):
    m, kc = g // NCH, g % NCH
    rows = pl.ds(RING0 + b * PRB, PRB)
    part = _dot(_bf(xnp[kc, pl.ds(b * (PRB // 2), PRB // 2), :]),
                _bf(wsrc[m * H + h, _pk_rows(g, 0, DCH // 2), :]))
    dst = qkvbuf[h].at[m]
    if may_be_first and isinstance(g, int):
      dst[rows, :] = part if kc == 0 else dst[rows, :] + part
      return
    old = dst[rows, :]
    if may_be_first:
      old = jnp.where(kc == 0, np.float32(0), old)
    dst[rows, :] = old + part

  NB = XP // PRB

  def pro_half(g, wsrc, half, may_be_first):
    for b in range(half * NB // 2, (half + 1) * NB // 2):
      for h in range(H):
        pro_dot(g, wsrc, may_be_first, b, h)

  NG = 3 * NCH

  def stage_wait_if(g):
    pl.when(g < NG)(lambda: stage_wait(g))

  stage_wait(0)
  for g in range(1, NSLOT):
    stage_start(g)
  relayout(0, wqa)
  stage_start(NSLOT)
  ln_pro(0)
  for b in range(NB):
    if b + 1 < NB:
      ln_pro(b + 1)
    for h in range(H):
      pro_dot(0, wqa, True, b, h)
  stage_wait(1)
  relayout(1, wqb)
  stage_start(NSLOT + 1)
  pro_half(1, wqb, 0, False)
  stage_wait(2)
  stage_wait(3)

  def pro_body(i, _):
    g = 2 * i + 1
    pro_half(g, wqb, 1, False)
    relayout(g + 1, wqa)
    pro_half(g + 1, wqa, 0, True)
    pro_half(g + 1, wqa, 1, True)
    relayout(g + 2, wqb)
    pro_half(g + 2, wqb, 0, False)
    stage_start(g + NSLOT + 1)
    stage_start(g + NSLOT + 2)

    @pl.when(i < 8)
    def _():
      for name, j in (("wo", i), ("w1", i), ("w2", i), ("w3", 2 * i), ("w3", 2 * i + 1)):
        strip(name, j).start()

    @pl.when(i == 8)
    def _():
      xb_cp.start()
      for j in range(16, 24):
        strip("w3", j).start()

    @pl.when(i == 9)
    def _():
      for j in range(24, 28):
        strip("w3", j).start()
      for j in range(4):
        strip("w4", j).start()

    @pl.when(i == 10)
    def _():
      for j in range(4, 8):
        strip("w4", j).start()

    stage_wait_if(g + 3)
    stage_wait_if(g + 4)
    return 0

  lax.fori_loop(0, NG // 2 - 1, pro_body, 0)

  def late_pro(k):
    b = NB // 2 + k
    return lambda j: [pro_dot(NG - 1, wqb, False, b, h) for h in range(j * 4, j * 4 + 4)]

  row = lax.broadcasted_iota(jnp.int32, (L, L), 0)
  col = lax.broadcasted_iota(jnp.int32, (L, L), 1)
  mask = (row < M) | (col <= row)

  def st_xn(s):
    xs = xv[_rows(XP + s * RX, RX), :].astype(f32)
    xnbuf[s % 2] = _ln(xs)

  def wrow(s):
    return _rows(((s + (XP + RING0) // RX) % (RING // RX)) * RX, RX)

  def rrow(s):
    return _rows(((s + RING0 // seg) % (RING // seg)) * seg, seg)

  def st_lhs(s):
    return jnp.concatenate([membuf[...], xnbuf[s % 2]], axis=0).astype(bf16)

  def st_qkv(s, lhs, h, m):
    half = DCH // 2
    w = jnp.concatenate(
        [(wqa, wqb)[kc % 2][m * H + h, pl.ds((kc // 2) * half, half), :]
         for kc in range(NCH)], axis=0)
    r = _dot(lhs, _bf(w))
    qkvbuf[h][m, wrow(s), :] = r[M:]
    return r[:M]

  def ld(s, h, m, fresh):
    return jnp.concatenate([fresh, qkvbuf[h][m, rrow(s), :]], axis=0)

  def st_scores(q, k):
    return _dot_nt(q, k.astype(bf16))

  def st_softmax(sc):
    t = jnp.where(mask, sc * np.float32(scale * LOG2E), np.float32(-1e9 * LOG2E))
    e = jnp.exp2(t - jnp.max(t, axis=-1, keepdims=True))
    l = jnp.sum(e, axis=-1, keepdims=True)
    r = pl.reciprocal(l, approx=True)
    r = r * (2.0 - l * r)
    return e * r

  def st_pv(h, p, v):
    obuf[:, h * E:(h + 1) * E] = _dot(p, v.astype(bf16))

  def st_wo(s, j):
    r = _dot(obuf[...], _bf(wo[j]))
    membuf[:, j * 128:(j + 1) * 128] = r[:M]
    abuf[:, j * 128:(j + 1) * 128] = r[M:]

  def st_post(t):
    xs = xv[_rows(t * seg, seg), :].astype(f32)
    ha = xs + abuf[...]
    habuf[t % 4] = ha
    y = _ln(ha)
    ybuf[t % 4] = y
    zbuf[0] = _pk(_ln(y))

  def st_b1(t, j):
    g = _gelu(_dot(_bf(zbuf[0]), _bf(w1[j])))
    h1buf[_rows(PAD + t * seg, seg), j * 128:(j + 1) * 128] = g

  c4 = D // 4

  def st_shift(t, u):
    win = h1buf[_rows(t * seg, seg + 2 * PAD), :]
    g0 = win[PAD - 1:PAD - 1 + seg, 0 * c4:1 * c4]
    g1 = win[PAD + 1:PAD + 1 + seg, 1 * c4:2 * c4]
    g2 = win[PAD - 2:PAD - 2 + seg, 2 * c4:3 * c4]
    g3 = win[PAD + 2:PAD + 2 + seg, 3 * c4:4 * c4]
    zbuf[1 + 2 * u] = _pk(jnp.concatenate([g0, g1, g2, g3], axis=1))

  def st_b2(t, u, j):
    cs = slice(j * 128, (j + 1) * 128)
    x1buf[u, :, cs] = ybuf[t % 4, :, cs] + _dot(_bf(zbuf[1 + 2 * u]), _bf(w2[j]))

  def st_ln2(t, u):
    zbuf[2 + 2 * u] = _pk(_ln(x1buf[u]))

  def st_b3(t, u, j):
    gbuf[u, :, j * 128:(j + 1) * 128] = _pk(_gelu(_dot(_bf(zbuf[2 + 2 * u]), _bf(w3[j]))))

  def st_b4(t, u, j):
    cs = slice(j * 128, (j + 1) * 128)
    h2 = _dot(_bf(gbuf[u]), _bf(w4[j]))
    res = habuf[t % 4, :, cs] + (x1buf[u, :, cs] + h2)
    outv[_rows(t * seg, seg), cs] = res.astype(outv.dtype)

  def st_out(t):
    r = _rows(t * seg, seg)
    pltpu.make_async_copy(outv.at[r], out_hbm.at[r], sems.at[7]).start()

  def b_ops(t, u, suffix=""):
    ops = dict(SHIFT=lambda _: st_shift(t, u), B2=lambda j: st_b2(t, u, j),
               LN2=lambda _: st_ln2(t, u), B3=lambda j: st_b3(t, u, j),
               B4=lambda j: st_b4(t, u, j), OUT=lambda _: st_out(t))
    return {k + suffix: v for k, v in ops.items()}

  def run(schedule, ops):
    for tok in schedule.split():
      name, _, rng = tok.partition(":")
      lo, hi = map(int, rng.split("-")) if rng else (0, 1)
      if name in ops:
        for i in range(lo, hi):
          ops[name](i)

  def step(s, do_b1, do_b2, filler=None):
    t1, t2 = s - 1, s - 2
    ops = {}

    fresh, probs = {}, {}
    lhs = st_lhs(s)

    def op_q(h):
      fresh[h] = [st_qkv(s, lhs, h, m) for m in range(3)]

    def op_s(h):
      probs[h] = st_scores(ld(s, h, 0, fresh[h][0]), ld(s, h, 1, fresh[h][1]))

    def op_p(h):
      st_pv(h, st_softmax(probs.pop(h)), ld(s, h, 2, fresh.pop(h)[2]))

    def op_xn(_):
      st_xn(s + 1 if isinstance(s, int) else jnp.minimum(s + 1, nseg - 1))

    ops.update(Q=op_q, S=op_s, P=op_p, XN=op_xn, WO=lambda j: st_wo(s, j))

    if do_b1:
      ops.update(POST=lambda _: st_post(t1), B1=lambda j: st_b1(t1, j))

    if do_b2:
      ops.update(b_ops(t2, 0))
    elif filler is not None:
      ops.update(B4=filler)

    run(SCHEDULE, ops)

  xb_cp.wait()
  for cp in strips("wo") + strips("w1"):
    cp.wait()
  st_xn(0)
  assert NB == 4
  step(0, False, False, late_pro(0))
  step(1, True, False, late_pro(1))
  for cp in strips("w2") + strips("w3") + strips("w4"):
    cp.wait()

  def body(s, _):
    step(s, True, True)
    return 0

  lax.fori_loop(2, nseg, body, 0)
  t = nseg - 1
  ops = dict(POST=lambda _: st_post(t), B1=lambda j: st_b1(t, j))
  ops.update(b_ops(t - 1, 0, "a"))
  ops.update(b_ops(t, 1, "b"))
  run(DRAIN, ops)
  pltpu.make_async_copy(outv, out_hbm, sems.at[7]).wait()


def _forward(A_x, A_mem0, A_Wq, A_Wk, A_Wv, A_Wo, seg, B_w1, B_w2, B_w3, B_w4):
  assert A_x.shape == (1, S, D) and A_mem0.shape == (1, M, D)
  assert A_Wq.shape == (D, H, E) and A_Wo.shape == (H, E, D) and B_w3.shape == (D, F)
  assert seg == SEG and XP + (S // seg) * RX == S
  x2 = A_x.reshape(S, D)
  mem0 = A_mem0.reshape(M, D)
  wq, wk, wv = A_Wq, A_Wk, A_Wv
  wo = A_Wo.reshape(H * E, D)
  any_spec = pl.BlockSpec(memory_space=pl.ANY)
  scratch = [
      pltpu.VMEM((S, D), bf16),
      pltpu.VMEM((M, D), bf16),
      pltpu.VMEM((3 * H, D // 4, E), u32),
      pltpu.VMEM((3 * H, D // 4, E), u32),
      pltpu.VMEM((D // 128, H * E // 2, 128), u32),
      pltpu.VMEM((D // 128, D // 2, 128), u32),
      pltpu.VMEM((D // 128, D // 2, 128), u32),
      pltpu.VMEM((F // 128, D // 2, 128), u32),
      pltpu.VMEM((D // 128, F // 2, 128), u32),
      pltpu.VMEM((NSLOT, DCH, H // 2, E), u32),
      pltpu.VMEM((NCH, XP // 2, 128), u32),
      [pltpu.VMEM((3, RING, E), f32) for _ in range(H)],
      pltpu.VMEM((M, D), f32),
      pltpu.VMEM((2, RX, D), f32),
      pltpu.VMEM((M + seg, H * E), f32),
      pltpu.VMEM((seg, D), f32),
      pltpu.VMEM((4, seg, D), f32),
      pltpu.VMEM((4, seg, D), f32),
      pltpu.VMEM((S + 2 * PAD, D), f32),
      pltpu.VMEM((2, seg, D), f32),
      pltpu.VMEM((5, seg // 2, D), u32),
      pltpu.VMEM((2, seg // 2, F), u32),
      pltpu.VMEM((S, D), A_x.dtype),
      pltpu.SemaphoreType.DMA((NSLOT,)),
      pltpu.SemaphoreType.DMA((12,)),
  ]
  out = pl.pallas_call(
      functools.partial(_kernel, seg),
      out_shape=jax.ShapeDtypeStruct((S, D), A_x.dtype),
      in_specs=[any_spec] * 10,
      out_specs=any_spec,
      scratch_shapes=scratch,
      compiler_params=pltpu.CompilerParams(vmem_limit_bytes=126 * 2**20),
  )(x2, mem0, wq, wk, wv, wo, B_w1, B_w2, B_w3, B_w4)
  return out.reshape(1, S, D)


def pallas_sequential_preLN__memory_aug_recurrent_mem_tr__mixer_s_mlp__prompt_kernel(
    A_x, A_mem0, A_Wq, A_Wk, A_Wv, A_Wo, A_seg_len, B_x, B_w1, B_w2, B_w3, B_w4):
  del B_x
  seg = int(A_seg_len) if isinstance(A_seg_len, (int, np.integer)) else SEG
  return _forward(A_x, A_mem0, A_Wq, A_Wk, A_Wv, A_Wo, seg, B_w1, B_w2, B_w3, B_w4)
```
